```python
import jax
import jax.numpy as jnp

def _softmax(x, axis=-1):
    return jax.nn.softmax(x, axis=axis)

def _gelu(x):
    return jax.nn.gelu(x, approximate=True)

def _silu(x):
    return jax.nn.silu(x)

def _sigmoid(x):
    return jax.nn.sigmoid(x)

def _layernorm(x, axis=-1, eps=1e-05):
    m = jnp.mean(x, axis=axis, keepdims=True)
    v = jnp.var(x, axis=axis, keepdims=True)
    return (x - m) / jnp.sqrt(v + eps)

def _scatter_add(tgt, idx, src, axis=0):
    return tgt.at[idx].add(src)

def _segment_sum(src, seg, n):
    return jax.ops.segment_sum(src, seg, n)

class _Rng:

    def __init__(self, key):
        self._k = key

    def _next(self):
        self._k, sub = jax.random.split(self._k)
        return sub

    def normal(self, shape):
        return jax.random.normal(self._next(), shape, dtype=jnp.bfloat16)

    def randint(self, lo, hi, shape):
        return jax.random.randint(self._next(), shape, lo, hi, dtype=jnp.int32)

    def uniform(self, shape, lo=0.0, hi=1.0):
        return jax.random.uniform(self._next(), shape, jnp.bfloat16, lo, hi)

    def permutation(self, n):
        return jax.random.permutation(self._next(), n)
kernel_name = 'gated_mix__memory_aug_recurrent_mem_tr__sliding_local_dilated__prompt'

def setup_inputs():
    _rng = _Rng(jax.random.key(int.from_bytes(__import__("os").urandom(4), "little")))
    _w = lambda a: (lambda t: t.astype(jnp.bfloat16) if jnp.issubdtype(t.dtype, jnp.floating) else t)(jnp.asarray(a))

    def _A_setup():
        B, S, Dm = (1, 2048, 640)
        H, Dh = (32, 192)
        M, seg = (8, 32)
        seg = min(seg, S)
        S = S // seg * seg
        return {'x': _w((lambda *s: _rng.normal(s) * 0.05)(B, S, Dm)), 'mem0': _w((lambda *s: _rng.normal(s) * 0.05)(B, M, Dm)), 'Wq': _w((lambda *s: _rng.normal(s) * 0.05)(Dm, H, Dh) * Dm ** (-0.5)), 'Wk': _w((lambda *s: _rng.normal(s) * 0.05)(Dm, H, Dh) * Dm ** (-0.5)), 'Wv': _w((lambda *s: _rng.normal(s) * 0.05)(Dm, H, Dh) * Dm ** (-0.5)), 'Wo': _w((lambda *s: _rng.normal(s) * 0.05)(H, Dh, Dm) * (H * Dh) ** (-0.5)), 'seg_len': seg}
    _A_in = _A_setup()

    def _B_setup():
        B, S, D = (1, 2048, 640)
        return {'x': _w((lambda *s: _rng.normal(s) * 0.05)(B, S, D)), 'wqkv': _w((lambda *s: _rng.normal(s) * 0.05)(D, 3 * D)), 'wo': _w((lambda *s: _rng.normal(s) * 0.05)(D, D))}
    _B_in = _B_setup()
    return {'A_x': _A_in['x'], 'A_mem0': _A_in['mem0'], 'A_Wq': _A_in['Wq'], 'A_Wk': _A_in['Wk'], 'A_Wv': _A_in['Wv'], 'A_Wo': _A_in['Wo'], 'A_seg_len': _A_in['seg_len'], 'B_x': _B_in['x'], 'B_wqkv': _B_in['wqkv'], 'B_wo': _B_in['wo'], 'gate_w': _w((lambda *s: _rng.normal(s) * 0.05)(640))}

def reference(A_x, A_mem0, A_Wq, A_Wk, A_Wv, A_Wo, A_seg_len, B_x, B_wqkv, B_wo, gate_w):

    def _A_ref(x, mem0, Wq, Wk, Wv, Wo, seg_len):
        B, S, Dm = x.shape
        H, Dh = (Wq.shape[1], Wq.shape[2])
        M = mem0.shape[1]
        scale = Dh ** (-0.5)
        n_seg = S // seg_len
        L = M + seg_len
        idx = jnp.arange(L)
        mask = (idx[:, None] < M) | (idx[:, None] >= idx[None, :])
        mem = mem0
        outs = []
        for s in range(n_seg):
            xs = x[:, s * seg_len:(s + 1) * seg_len, :].copy()
            h = jnp.concatenate([mem, xs], axis=1)
            q = jnp.einsum('btd,dhe->bhte', h, Wq)
            k = jnp.einsum('btd,dhe->bhte', h, Wk)
            v = jnp.einsum('btd,dhe->bhte', h, Wv)
            scores = jnp.einsum('bhqe,bhke->bhqk', q, k) * scale
            scores = jnp.where(mask[None, None], scores, -1000000000.0)
            p = _softmax(scores, axis=-1)
            o = jnp.einsum('bhqk,bhke->bhqe', p, v)
            o = jnp.einsum('bhte,hed->btd', o, Wo)
            mem = o[:, :M, :].copy()
            outs.append(o[:, M:, :])
        return jnp.concatenate(outs, axis=1)

    def _B_ref(x, wqkv, wo):
        B, S, D = x.shape
        H = 32
        Dh = D // H
        W, dil = (8, 2)
        qkv = (lambda x, *d: x.transpose(*d))((x @ wqkv).reshape(B, S, 3, H, Dh), 2, 0, 3, 1, 4)
        q, k, v = (qkv[0], qkv[1], qkv[2])
        scale = Dh ** (-0.5)
        pos = jnp.arange(S)
        off = jnp.arange(W) * dil
        idx = pos[:, None] - off[None, :]
        mask = idx >= 0
        idx_c = jnp.where(mask, idx, 0).reshape(-1)
        kg = k[:, :, idx_c, :].reshape(B, H, S, W, Dh)
        vg = v[:, :, idx_c, :].reshape(B, H, S, W, Dh)
        logits = jnp.einsum('bhsd,bhswd->bhsw', q, kg) * scale
        logits = jnp.where(mask[None, None, :, :], logits, -1000000000.0)
        attn = _softmax(logits, axis=-1)
        o = jnp.einsum('bhsw,bhswd->bhsd', attn, vg)
        return (lambda x, *d: x.transpose(*d))(o, 0, 2, 1, 3).reshape(B, S, D) @ wo
    x = A_x
    g = _sigmoid((x * gate_w).sum(-1, keepdims=True))
    a = _A_ref(x, A_mem0, A_Wq, A_Wk, A_Wv, A_Wo, A_seg_len)
    b = _B_ref(x, B_wqkv, B_wo)
    return g * a + (1 - g) * b
```

```python
import functools

import jax
import jax.numpy as jnp
from jax import lax
import jax.experimental.pallas as pl
import jax.experimental.pallas.tpu as pltpu

F32 = jnp.float32
BF16 = jnp.bfloat16
LANES = 128
NEG = -1000000000.0

B_HEADS = 32
B_WIN = 8
B_DIL = 2
B_PAD = 16
B_CHUNK = 256
B_SUB = 32


def _dot(a, b):
    return lax.dot_general(a, b, (((1,), (0,)), ((), ())),
                           preferred_element_type=F32)


def _dot_nt(a, b):
    return lax.dot_general(a, b, (((1,), (1,)), ((), ())),
                           preferred_element_type=F32)


def _kernel(x_hbm, mem0_ref, wq_hbm, wk_hbm, wv_hbm, wo_hbm, bqkv_hbm, bwo_hbm,
            gate_ref, out_hbm,
            x_v, wraw, w_v, wo_v, bqkv_v, bwo_v, slab, bqkv_p, bwo_p,
            q_s, k_s, v_s, ob_s, g_v, gb_v, out_v, sem_in, sem_w, sem_out,
            *, seg, n_heads, dh):
    S, D = x_v.shape
    M = mem0_ref.shape[0]
    L = M + seg
    n_seg = S // seg
    n_pair = n_heads // 2
    PW = 2 * dh
    n_slab = D // LANES
    bdh = D // B_HEADS
    n_chunk = S // B_CHUNK
    ppc = n_pair // n_chunk

    cp_bqkv = pltpu.make_async_copy(bqkv_hbm, bqkv_v, sem_in.at[0])
    cp_x = pltpu.make_async_copy(x_hbm, x_v, sem_in.at[1])
    cp_bwo = pltpu.make_async_copy(bwo_hbm, bwo_v, sem_in.at[2])
    cp_wo = pltpu.make_async_copy(wo_hbm, wo_v, sem_in.at[3])

    def cp_w(c, j):
        rows = pl.ds(c * ppc * PW, ppc * PW)
        src = (wq_hbm, wk_hbm, wv_hbm)[j]
        return pltpu.make_async_copy(src.at[rows], wraw.at[j, rows],
                                     sem_w.at[c, j])

    cp_bqkv.start()
    cp_x.start()
    cp_bwo.start()
    for c in range(n_chunk):
        for j in range(3):
            cp_w(c, j).start()
    cp_wo.start()

    cp_bqkv.wait()
    for s in range(n_slab):
        slab[s] = bqkv_v[s * LANES:(s + 1) * LANES, :].astype(F32).T
    for part in range(3):
        for d in range(bdh):
            r0 = part * D + d * B_HEADS
            for s in range(n_slab):
                bqkv_p[r0:r0 + B_HEADS, s * LANES:(s + 1) * LANES] = slab[
                    s, pl.ds(part * D + d, B_HEADS, stride=bdh), :].astype(BF16)
    cp_bwo.wait()
    for s in range(n_slab):
        slab[s, 0:D, :] = bwo_v[:, s * LANES:(s + 1) * LANES].astype(F32)
    for d in range(bdh):
        for s in range(n_slab):
            bwo_p[d * B_HEADS:(d + 1) * B_HEADS, s * LANES:(s + 1) * LANES] = slab[
                s, pl.ds(d, B_HEADS, stride=bdh), :].astype(BF16)
    cp_x.wait()

    bscale = bdh ** -0.5
    gate = gate_ref[...].astype(F32)

    def b_chunk(c, carry):
        t0 = pl.multiple_of(c * B_CHUNK, B_CHUNK)
        xc = x_v[pl.ds(t0, B_CHUNK), :]
        qkv = _dot_nt(xc, bqkv_p[...])

        @pl.when(c == 0)
        def _():
            for s in range(n_slab):
                k_s[s, B_CHUNK:, :] = jnp.broadcast_to(
                    qkv[0:1, D + s * LANES:D + (s + 1) * LANES], (B_PAD, LANES))
                v_s[s, B_CHUNK:, :] = jnp.broadcast_to(
                    qkv[0:1, 2 * D + s * LANES:2 * D + (s + 1) * LANES],
                    (B_PAD, LANES))

        for s in range(n_slab):
            k_s[s, 0:B_PAD, :] = k_s[s, B_CHUNK:, :]
            v_s[s, 0:B_PAD, :] = v_s[s, B_CHUNK:, :]
            q_s[s] = qkv[:, s * LANES:(s + 1) * LANES]
            k_s[s, B_PAD:, :] = qkv[:, D + s * LANES:D + (s + 1) * LANES]
            v_s[s, B_PAD:, :] = qkv[:, 2 * D + s * LANES:2 * D + (s + 1) * LANES]

        for r in range(0, B_CHUNK, B_SUB):
            qs = [q_s[s, r:r + B_SUB, :] for s in range(n_slab)]
            logits = []
            for w in range(B_WIN):
                o = B_PAD + r - w * B_DIL
                acc = qs[0] * k_s[0, o:o + B_SUB, :]
                for s in range(1, n_slab):
                    acc = acc + qs[s] * k_s[s, o:o + B_SUB, :]
                acc = acc + pltpu.roll(acc, 64, 1)
                acc = acc + pltpu.roll(acc, 32, 1)
                acc = acc * bscale
                if r < w * B_DIL:
                    pos = t0 + r + lax.broadcasted_iota(
                        jnp.int32, (B_SUB, LANES), 0)
                    acc = jnp.where(pos >= w * B_DIL, acc, NEG)
                logits.append(acc)
            mx = functools.reduce(jnp.maximum, logits)
            es = [jnp.exp(l - mx) for l in logits]
            inv = 1.0 / functools.reduce(jnp.add, es)
            for s in range(n_slab):
                acc = None
                for w in range(B_WIN):
                    o = B_PAD + r - w * B_DIL
                    t = es[w] * v_s[s, o:o + B_SUB, :]
                    acc = t if acc is None else acc + t
                ob_s[r:r + B_SUB, s * LANES:(s + 1) * LANES] = (
                    acc * inv).astype(BF16)

        b = _dot(ob_s[...], bwo_p[...])
        g = jax.nn.sigmoid(
            jnp.sum(xc.astype(F32) * gate, axis=-1, keepdims=True))
        g_v[pl.ds(t0, B_CHUNK), :] = jnp.broadcast_to(g, (B_CHUNK, LANES))
        gb_v[pl.ds(t0, B_CHUNK), :] = (1.0 - g) * b

        for j in range(3):
            cp_w(c, j).wait()
            for i in range(ppc):
                p = c * ppc + i
                rows = pl.ds(pl.multiple_of(p * PW, PW), PW)
                w_v[p, :, j * PW:(j + 1) * PW] = wraw[j, rows, :].T
        return carry

    lax.fori_loop(0, n_chunk, b_chunk, 0)
    cp_wo.wait()

    scale = dh ** -0.5

    def step(s, mem):
        r0 = pl.multiple_of(s * seg, seg)
        h = jnp.concatenate([mem, x_v[pl.ds(r0, seg), :].astype(F32)], axis=0)

        row = lax.broadcasted_iota(jnp.int32, (L, 2 * L), 0)
        col = lax.broadcasted_iota(jnp.int32, (L, 2 * L), 1)
        first = col < L
        visible = (row < M) | (row >= jnp.where(first, col, col - L))
        lo = lax.broadcasted_iota(jnp.int32, (L, PW), 1) < dh

        def block_diag(t):
            return jnp.concatenate(
                [jnp.where(lo, t, 0.0), jnp.where(lo, 0.0, t)],
                axis=0).astype(BF16)

        def project(p):
            qkv = _dot(h, w_v[p])
            return (qkv[:, :PW], block_diag(qkv[:, PW:2 * PW]),
                    block_diag(qkv[:, 2 * PW:]))

        def scores(q, kb):
            sc = jnp.where(visible, _dot_nt(q, kb) * scale, NEG)
            ma = jnp.max(jnp.where(first, sc, -jnp.inf), axis=-1, keepdims=True)
            mb = jnp.max(jnp.where(first, -jnp.inf, sc), axis=-1, keepdims=True)
            e = jnp.exp(sc - jnp.where(first, ma, mb))
            sa = jnp.sum(jnp.where(first, e, 0.0), axis=-1, keepdims=True)
            sb = jnp.sum(jnp.where(first, 0.0, e), axis=-1, keepdims=True)
            return e * jnp.where(first, 1.0 / sa, 1.0 / sb)

        proj, prob, outs = {}, {}, {}
        for t in range(n_pair + 2):
            if t < n_pair:
                proj[t] = project(t)
            if 0 <= t - 1 < n_pair:
                prob[t - 1] = scores(proj[t - 1][0], proj[t - 1][1])
            if 0 <= t - 2 < n_pair:
                outs[t - 2] = _dot(prob[t - 2], proj[t - 2][2])
        acc = None
        for p in range(n_pair):
            y = _dot(outs[p], wo_v[p * PW:(p + 1) * PW, :])
            acc = y if acc is None else acc + y

        g = g_v[pl.ds(r0, seg), :]
        g = jnp.concatenate([g] * n_slab, axis=1)
        out_v[pl.ds(r0, seg), :] = (
            g * acc[M:] + gb_v[pl.ds(r0, seg), :]).astype(out_v.dtype)
        pltpu.make_async_copy(out_v.at[pl.ds(r0, seg)],
                              out_hbm.at[pl.ds(r0, seg)], sem_out.at[0]).start()
        return acc[:M]

    lax.fori_loop(0, n_seg, step, mem0_ref[...].astype(F32))
    pltpu.make_async_copy(out_v, out_v, sem_out.at[0]).wait()


@functools.partial(jax.jit, static_argnames=("A_seg_len",))
def pallas_gated_mix__memory_aug_recurrent_mem_tr__sliding_local_dilated__prompt_kernel(
    A_x: jax.Array,
    A_mem0: jax.Array,
    A_Wq: jax.Array,
    A_Wk: jax.Array,
    A_Wv: jax.Array,
    A_Wo: jax.Array,
    A_seg_len: int,
    B_x: jax.Array,
    B_wqkv: jax.Array,
    B_wo: jax.Array,
    gate_w: jax.Array,
):
    del B_x
    _, S, D = A_x.shape
    _, H, Dh = A_Wq.shape
    M = A_mem0.shape[1]
    seg = int(A_seg_len)
    n_pair = H // 2
    n_slab = D // LANES
    n_chunk = S // B_CHUNK

    def by_head(w):
        return jnp.transpose(w, (1, 2, 0)).reshape(H * Dh, D)

    hbm = pl.BlockSpec(memory_space=pl.ANY)
    vmem = pl.BlockSpec(memory_space=pltpu.VMEM)
    out = pl.pallas_call(
        functools.partial(_kernel, seg=seg, n_heads=H, dh=Dh),
        out_shape=jax.ShapeDtypeStruct((S, D), A_x.dtype),
        in_specs=[hbm, vmem, hbm, hbm, hbm, hbm, hbm, hbm, vmem],
        out_specs=hbm,
        scratch_shapes=[
            pltpu.VMEM((S, D), BF16),
            pltpu.VMEM((3, H * Dh, D), BF16),
            pltpu.VMEM((n_pair, D, 6 * Dh), BF16),
            pltpu.VMEM((H * Dh, D), BF16),
            pltpu.VMEM((D, 3 * D), BF16),
            pltpu.VMEM((D, D), BF16),
            pltpu.VMEM((n_slab, 3 * D, LANES), F32),
            pltpu.VMEM((3 * D, D), BF16),
            pltpu.VMEM((D, D), BF16),
            pltpu.VMEM((n_slab, B_CHUNK, LANES), F32),
            pltpu.VMEM((n_slab, B_CHUNK + B_PAD, LANES), F32),
            pltpu.VMEM((n_slab, B_CHUNK + B_PAD, LANES), F32),
            pltpu.VMEM((B_CHUNK, D), BF16),
            pltpu.VMEM((S, LANES), F32),
            pltpu.VMEM((S, D), F32),
            pltpu.VMEM((S, D), A_x.dtype),
            pltpu.SemaphoreType.DMA((4,)),
            pltpu.SemaphoreType.DMA((n_chunk, 3)),
            pltpu.SemaphoreType.DMA((1,)),
        ],
        compiler_params=pltpu.CompilerParams(
            vmem_limit_bytes=110 * 1024 * 1024),
    )(A_x.reshape(S, D), A_mem0.reshape(M, D), by_head(A_Wq), by_head(A_Wk),
      by_head(A_Wv), A_Wo.reshape(H * Dh, D), B_wqkv, B_wo,
      gate_w.reshape(1, D))
    return out.reshape(1, S, D)
```

```python
import functools

import jax
import jax.numpy as jnp
from jax import lax
import jax.experimental.pallas as pl
import jax.experimental.pallas.tpu as pltpu

F32 = jnp.float32
BF16 = jnp.bfloat16
LANES = 128
NEG = -1000000000.0

B_HEADS = 32
B_WIN = 8
B_DIL = 2
B_PAD = 16
B_CHUNK = 128
W_AHEAD = 2
B_SUB = 32


def _dot(a, b):
    return lax.dot_general(a, b, (((1,), (0,)), ((), ())),
                           preferred_element_type=F32)


def _dot_nt(a, b):
    return lax.dot_general(a, b, (((1,), (1,)), ((), ())),
                           preferred_element_type=F32)


def _kernel(x_hbm, mem0_ref, wq_hbm, wk_hbm, wv_hbm, wo_hbm, bqkv_hbm, bwo_hbm,
            gate_ref, out_hbm,
            x_v, wraw, w_v, wo_v, bqkv_v, bwo_v, slab, bqkv_p, bwo_p,
            q_a, k_a, v_a, q_b, k_b, v_b, g_v, gb_v, out_v,
            sem_in, sem_w, sem_out,
            *, seg, n_heads, dh):
    S, D = x_v.shape
    M = mem0_ref.shape[0]
    L = M + seg
    n_seg = S // seg
    n_pair = n_heads // 2
    PW = 2 * dh
    n_slab = D // LANES
    bdh = D // B_HEADS
    n_chunk = S // (2 * B_CHUNK)
    ppc = n_pair // n_chunk

    buf_a, buf_b = (q_a, k_a, v_a), (q_b, k_b, v_b)

    cp_bqkv = pltpu.make_async_copy(bqkv_hbm, bqkv_v, sem_in.at[0])
    cp_x = pltpu.make_async_copy(x_hbm, x_v, sem_in.at[1])
    cp_bwo = pltpu.make_async_copy(bwo_hbm, bwo_v, sem_in.at[2])
    cp_wo = pltpu.make_async_copy(wo_hbm, wo_v, sem_in.at[3])

    def cp_w(c, j):
        rows = pl.ds(pl.multiple_of(c * ppc * PW, PW), ppc * PW)
        src = (wq_hbm, wk_hbm, wv_hbm)[j]
        return pltpu.make_async_copy(src.at[rows], wraw.at[j, rows],
                                     sem_w.at[c, j])

    cp_bqkv.start()
    cp_x.start()
    cp_bwo.start()

    cp_bqkv.wait()
    for c in range(W_AHEAD):
        for j in range(3):
            cp_w(c, j).start()
    for s in range(n_slab):
        slab[s] = bqkv_v[s * LANES:(s + 1) * LANES, :].astype(F32).T
    for part in range(3):
        for d in range(bdh):
            r0 = part * D + d * B_HEADS
            for s in range(n_slab):
                bqkv_p[r0:r0 + B_HEADS, s * LANES:(s + 1) * LANES] = slab[
                    s, pl.ds(part * D + d, B_HEADS, stride=bdh), :].astype(BF16)
    cp_bwo.wait()
    for s in range(n_slab):
        slab[s, 0:D, :] = bwo_v[:, s * LANES:(s + 1) * LANES].astype(F32)
    for d in range(bdh):
        for s in range(n_slab):
            bwo_p[d * B_HEADS:(d + 1) * B_HEADS, s * LANES:(s + 1) * LANES] = slab[
                s, pl.ds(d, B_HEADS, stride=bdh), :].astype(BF16)
    cp_x.wait()

    bscale = bdh ** -0.5
    gate = gate_ref[...].astype(F32)

    def b_project(t0, dst, prev):
        q_s, k_s, v_s = dst
        qkv = _dot_nt(x_v[pl.ds(t0, B_CHUNK), :], bqkv_p[...])
        for s in range(n_slab):
            q, k, v = (qkv[:, j * D + s * LANES:j * D + (s + 1) * LANES]
                       for j in range(3))
            q_s[s] = q
            k_s[s, B_PAD:, :] = k
            v_s[s, B_PAD:, :] = v
            if prev is None:
                k_s[s, 0:B_PAD, :] = jnp.broadcast_to(k[0:1], (B_PAD, LANES))
                v_s[s, 0:B_PAD, :] = jnp.broadcast_to(v[0:1], (B_PAD, LANES))
            else:
                k_s[s, 0:B_PAD, :] = prev[1][s, B_CHUNK:, :]
                v_s[s, 0:B_PAD, :] = prev[2][s, B_CHUNK:, :]

    def b_attend(t0, src):
        q_s, k_s, v_s = src
        blocks = []
        for r in range(0, B_CHUNK, B_SUB):
            qs = [q_s[s, r:r + B_SUB, :] for s in range(n_slab)]
            logits = []
            for w in range(B_WIN):
                o = B_PAD + r - w * B_DIL
                acc = qs[0] * k_s[0, o:o + B_SUB, :]
                for s in range(1, n_slab):
                    acc = acc + qs[s] * k_s[s, o:o + B_SUB, :]
                acc = acc + pltpu.roll(acc, 64, 1)
                acc = acc + pltpu.roll(acc, 32, 1)
                acc = acc * bscale
                if r < w * B_DIL:
                    pos = t0 + r + lax.broadcasted_iota(
                        jnp.int32, (B_SUB, LANES), 0)
                    acc = jnp.where(pos >= w * B_DIL, acc, NEG)
                logits.append(acc)
            mx = functools.reduce(jnp.maximum, logits)
            es = [jnp.exp(l - mx) for l in logits]
            inv = 1.0 / functools.reduce(jnp.add, es)
            cols = []
            for s in range(n_slab):
                acc = None
                for w in range(B_WIN):
                    o = B_PAD + r - w * B_DIL
                    t = es[w] * v_s[s, o:o + B_SUB, :]
                    acc = t if acc is None else acc + t
                cols.append((acc * inv).astype(BF16))
            blocks.append(jnp.concatenate(cols, axis=1))
        return jnp.concatenate(blocks, axis=0)

    def b_finish(t0, ob):
        rows = pl.ds(t0, B_CHUNK)
        g = jax.nn.sigmoid(jnp.sum(x_v[rows, :].astype(F32) * gate,
                                   axis=-1, keepdims=True))
        g_v[rows, :] = jnp.broadcast_to(g, (B_CHUNK, LANES))
        gb_v[rows, :] = (1.0 - g) * _dot(ob, bwo_p[...])

    b_project(0, buf_a, None)

    def b_body(c, carry):
        @pl.when(c + W_AHEAD < n_chunk)
        def _():
            for j in range(3):
                cp_w(c + W_AHEAD, j).start()

        @pl.when(c + W_AHEAD == n_chunk)
        def _():
            cp_wo.start()

        for j in range(3):
            cp_w(c, j).wait()

        def transpose_pair(p):
            rows = pl.ds(pl.multiple_of(p * PW, PW), PW)
            for j in range(3):
                w_v[p, :, j * PW:(j + 1) * PW] = wraw[j, rows, :].T

        t0 = pl.multiple_of(c * 2 * B_CHUNK, B_CHUNK)
        t1 = pl.multiple_of(t0 + B_CHUNK, B_CHUNK)
        t2 = pl.multiple_of(jnp.minimum(t1 + B_CHUNK, S - B_CHUNK), B_CHUNK)
        b_project(t1, buf_b, buf_a)
        ob = b_attend(t0, buf_a)
        for i in range(ppc // 2):
            transpose_pair(c * ppc + i)
        b_finish(t0, ob)
        b_project(t2, buf_a, buf_b)
        ob = b_attend(t1, buf_b)
        for i in range(ppc // 2, ppc):
            transpose_pair(c * ppc + i)
        b_finish(t1, ob)
        return carry

    lax.fori_loop(0, n_chunk, b_body, 0)
    cp_wo.wait()

    scale = dh ** -0.5

    def step(s, mem):
        r0 = pl.multiple_of(s * seg, seg)
        h = jnp.concatenate([mem, x_v[pl.ds(r0, seg), :].astype(F32)], axis=0)

        row = lax.broadcasted_iota(jnp.int32, (L, 2 * L), 0)
        col = lax.broadcasted_iota(jnp.int32, (L, 2 * L), 1)
        first = col < L
        visible = (row < M) | (row >= jnp.where(first, col, col - L))
        lo = lax.broadcasted_iota(jnp.int32, (L, PW), 1) < dh

        def block_diag(t):
            return jnp.concatenate(
                [jnp.where(lo, t, 0.0), jnp.where(lo, 0.0, t)],
                axis=0).astype(BF16)

        def project(p):
            qkv = _dot(h, w_v[p])
            return (qkv[:, :PW], block_diag(qkv[:, PW:2 * PW]),
                    block_diag(qkv[:, 2 * PW:]))

        def scores(q, kb):
            sc = jnp.where(visible, _dot_nt(q, kb) * scale, NEG)
            ma = jnp.max(jnp.where(first, sc, -jnp.inf), axis=-1, keepdims=True)
            mb = jnp.max(jnp.where(first, -jnp.inf, sc), axis=-1, keepdims=True)
            e = jnp.exp(sc - jnp.where(first, ma, mb))
            sa = jnp.sum(jnp.where(first, e, 0.0), axis=-1, keepdims=True)
            sb = jnp.sum(jnp.where(first, 0.0, e), axis=-1, keepdims=True)
            return e * jnp.where(first, 1.0 / sa, 1.0 / sb)

        proj, prob, outs = {}, {}, {}
        acc = None

        def out_proj(acc, pairs):
            for p in pairs:
                y = _dot(outs[p], wo_v[p * PW:(p + 1) * PW, :])
                acc = y if acc is None else acc + y
            return acc

        for t in range(n_pair + 2):
            if t < n_pair:
                proj[t] = project(t)
            if t == n_pair:
                acc = out_proj(acc, range(0, n_pair // 4))
            if 0 <= t - 1 < n_pair:
                prob[t - 1] = scores(proj[t - 1][0], proj[t - 1][1])
            if t == n_pair + 1:
                acc = out_proj(acc, range(n_pair // 4, n_pair - 4))
            if 0 <= t - 2 < n_pair:
                outs[t - 2] = _dot(prob[t - 2], proj[t - 2][2])
        acc = out_proj(acc, range(n_pair - 4, n_pair))

        g = g_v[pl.ds(r0, seg), :]
        g = jnp.concatenate([g] * n_slab, axis=1)
        out_v[pl.ds(r0, seg), :] = (
            g * acc[M:] + gb_v[pl.ds(r0, seg), :]).astype(out_v.dtype)
        pltpu.make_async_copy(out_v.at[pl.ds(r0, seg)],
                              out_hbm.at[pl.ds(r0, seg)], sem_out.at[0]).start()
        return acc[:M]

    lax.fori_loop(0, n_seg, step, mem0_ref[...].astype(F32))
    pltpu.make_async_copy(out_v, out_v, sem_out.at[0]).wait()


@functools.partial(jax.jit, static_argnames=("A_seg_len",))
def pallas_gated_mix__memory_aug_recurrent_mem_tr__sliding_local_dilated__prompt_kernel(
    A_x: jax.Array,
    A_mem0: jax.Array,
    A_Wq: jax.Array,
    A_Wk: jax.Array,
    A_Wv: jax.Array,
    A_Wo: jax.Array,
    A_seg_len: int,
    B_x: jax.Array,
    B_wqkv: jax.Array,
    B_wo: jax.Array,
    gate_w: jax.Array,
):
    del B_x
    _, S, D = A_x.shape
    _, H, Dh = A_Wq.shape
    M = A_mem0.shape[1]
    seg = int(A_seg_len)
    n_pair = H // 2
    n_slab = D // LANES
    n_chunk = S // (2 * B_CHUNK)

    def by_head(w):
        return jnp.transpose(w, (1, 2, 0)).reshape(H * Dh, D)

    qkv_buf = [pltpu.VMEM((n_slab, B_CHUNK, LANES), F32),
               pltpu.VMEM((n_slab, B_CHUNK + B_PAD, LANES), F32),
               pltpu.VMEM((n_slab, B_CHUNK + B_PAD, LANES), F32)]
    hbm = pl.BlockSpec(memory_space=pl.ANY)
    vmem = pl.BlockSpec(memory_space=pltpu.VMEM)
    out = pl.pallas_call(
        functools.partial(_kernel, seg=seg, n_heads=H, dh=Dh),
        out_shape=jax.ShapeDtypeStruct((S, D), A_x.dtype),
        in_specs=[hbm, vmem, hbm, hbm, hbm, hbm, hbm, hbm, vmem],
        out_specs=hbm,
        scratch_shapes=[
            pltpu.VMEM((S, D), BF16),
            pltpu.VMEM((3, H * Dh, D), BF16),
            pltpu.VMEM((n_pair, D, 6 * Dh), BF16),
            pltpu.VMEM((H * Dh, D), BF16),
            pltpu.VMEM((D, 3 * D), BF16),
            pltpu.VMEM((D, D), BF16),
            pltpu.VMEM((n_slab, 3 * D, LANES), F32),
            pltpu.VMEM((3 * D, D), BF16),
            pltpu.VMEM((D, D), BF16),
            *qkv_buf, *qkv_buf,
            pltpu.VMEM((S, LANES), F32),
            pltpu.VMEM((S, D), F32),
            pltpu.VMEM((S, D), A_x.dtype),
            pltpu.SemaphoreType.DMA((4,)),
            pltpu.SemaphoreType.DMA((n_chunk, 3)),
            pltpu.SemaphoreType.DMA((1,)),
        ],
        compiler_params=pltpu.CompilerParams(
            vmem_limit_bytes=110 * 1024 * 1024),
    )(A_x.reshape(S, D), A_mem0.reshape(M, D), by_head(A_Wq), by_head(A_Wk),
      by_head(A_Wv), A_Wo.reshape(H * Dh, D), B_wqkv, B_wo,
      gate_w.reshape(1, D))
    return out.reshape(1, S, D)
```

```python
import functools

import jax
import jax.numpy as jnp
from jax import lax
import jax.experimental.pallas as pl
import jax.experimental.pallas.tpu as pltpu

F32 = jnp.float32
BF16 = jnp.bfloat16
LANES = 128
NEG = -1000000000.0

B_HEADS = 32
B_WIN = 8
B_DIL = 2
B_PAD = 16
B_CHUNK = 128
W_AHEAD = 2
PRE = 8
UNROLL = 1
B_SUB = 32


def _dot(a, b):
    return lax.dot_general(a, b, (((1,), (0,)), ((), ())),
                           preferred_element_type=F32)


def _dot_nt(a, b):
    return lax.dot_general(a, b, (((1,), (1,)), ((), ())),
                           preferred_element_type=F32)


def _kernel(x_hbm, mem0_ref, wq_hbm, wk_hbm, wv_hbm, wo_hbm, bqkv_hbm, bwo_hbm,
            gate_ref, out_hbm,
            x_v, xt_v, wraw, w_v, wo_v, bqkv_v, bwo_v, slab, bqkv_p, bwo_p,
            q_a, k_a, v_a, q_b, k_b, v_b, g_v, ob_v, b_v, qpre, out_v,
            sem_in, sem_b, sem_w, sem_out,
            *, seg, n_heads, dh):
    S, D = x_v.shape
    M = mem0_ref.shape[0]
    L = M + seg
    n_seg = S // seg
    n_pair = n_heads // 2
    PW = 2 * dh
    n_slab = D // LANES
    bdh = D // B_HEADS
    n_chunk = S // (2 * B_CHUNK)
    ppc = n_pair // n_chunk
    buf_a, buf_b = (q_a, k_a, v_a), (q_b, k_b, v_b)

    cp_x = pltpu.make_async_copy(x_hbm, x_v, sem_in.at[0])
    cp_bwo = pltpu.make_async_copy(bwo_hbm, bwo_v, sem_in.at[1])
    cp_wo = pltpu.make_async_copy(wo_hbm, wo_v, sem_in.at[2])

    def cp_bqkv(s):
        rows = pl.ds(s * LANES, LANES)
        return pltpu.make_async_copy(bqkv_hbm.at[rows], bqkv_v.at[rows],
                                     sem_b.at[s])

    def cp_w(c, j):
        rows = pl.ds(pl.multiple_of(c * ppc * PW, PW), ppc * PW)
        src = (wq_hbm, wk_hbm, wv_hbm)[j]
        return pltpu.make_async_copy(src.at[rows], wraw.at[j, rows],
                                     sem_w.at[c, j])

    for s in range(n_slab):
        cp_bqkv(s).start()
    cp_x.start()
    for ref in buf_b:
        ref[...] = jnp.zeros(ref.shape, ref.dtype)

    for s in range(n_slab):
        cp_bqkv(s).wait()
        if s == n_slab - 1:
            for c in range(W_AHEAD):
                for j in range(3):
                    cp_w(c, j).start()
            cp_bwo.start()
        slab[s] = bqkv_v[s * LANES:(s + 1) * LANES, :].astype(F32).T
        for part in range(3):
            for d in range(bdh):
                r0 = part * D + d * B_HEADS
                bqkv_p[r0:r0 + B_HEADS, s * LANES:(s + 1) * LANES] = slab[
                    s, pl.ds(part * D + d, B_HEADS, stride=bdh), :].astype(BF16)
    cp_x.wait()
    for i in range(0, n_seg, 2):
        xt_v[i * PRE:(i + 2) * PRE, :] = jnp.concatenate(
            [x_v[(i + u + 1) * seg - 2 * PRE:(i + u + 1) * seg, :]
             .astype(F32)[PRE:] for u in range(2)], axis=0).astype(BF16)

    bscale = bdh ** -0.5
    gate = gate_ref[...].astype(F32)

    def b_project(t0, dst, prev, is_first):
        qkv = _dot_nt(x_v[pl.ds(t0, B_CHUNK), :], bqkv_p[...])
        for s in range(n_slab):
            for j in range(3):
                t = qkv[:, j * D + s * LANES:j * D + (s + 1) * LANES]
                if j == 0:
                    dst[j][s] = t
                    continue
                halo = prev[j][s, B_CHUNK:, :]
                if is_first is not None:
                    halo = jnp.where(
                        is_first, jnp.broadcast_to(t[0:1], halo.shape), halo)
                dst[j][s, 0:B_PAD, :] = halo
                dst[j][s, B_PAD:, :] = t

    def b_attend(t0, src):
        q_s, k_s, v_s = src
        blocks = []
        for r in range(0, B_CHUNK, B_SUB):
            qs = [q_s[s, r:r + B_SUB, :] for s in range(n_slab)]
            logits = []
            for w in range(B_WIN):
                o = B_PAD + r - w * B_DIL
                acc = qs[0] * k_s[0, o:o + B_SUB, :]
                for s in range(1, n_slab):
                    acc = acc + qs[s] * k_s[s, o:o + B_SUB, :]
                acc = acc + pltpu.roll(acc, 64, 1)
                acc = acc + pltpu.roll(acc, 32, 1)
                acc = acc * bscale
                if r < w * B_DIL:
                    pos = t0 + r + lax.broadcasted_iota(
                        jnp.int32, (B_SUB, LANES), 0)
                    acc = jnp.where(pos >= w * B_DIL, acc, NEG)
                logits.append(acc)
            mx = functools.reduce(jnp.maximum, logits)
            es = [jnp.exp(l - mx) for l in logits]
            inv = 1.0 / functools.reduce(jnp.add, es)
            cols = []
            for s in range(n_slab):
                acc = None
                for w in range(B_WIN):
                    o = B_PAD + r - w * B_DIL
                    t = es[w] * v_s[s, o:o + B_SUB, :]
                    acc = t if acc is None else acc + t
                cols.append((acc * inv).astype(BF16))
            blocks.append(jnp.concatenate(cols, axis=1))
        rows = pl.ds(t0, B_CHUNK)
        ob_v[rows, :] = jnp.concatenate(blocks, axis=0)
        g = jax.nn.sigmoid(jnp.sum(x_v[rows, :].astype(F32) * gate,
                                   axis=-1, keepdims=True))
        g_v[rows, :] = jnp.broadcast_to(g, (B_CHUNK, LANES))

    def prepare_pair(p):
        rows = pl.ds(pl.multiple_of(p * PW, PW), PW)
        qpre[p] = _dot_nt(xt_v[...], wraw[0, rows, :])
        for j in range(3):
            w_v[p, :, j * PW:(j + 1) * PW] = wraw[j, rows, :].T

    def b_body(c, carry):
        @pl.when(c + W_AHEAD < n_chunk)
        def _():
            for j in range(3):
                cp_w(c + W_AHEAD, j).start()

        @pl.when(c + W_AHEAD == n_chunk)
        def _():
            cp_wo.start()

        t0 = pl.multiple_of(c * 2 * B_CHUNK, B_CHUNK)
        t1 = pl.multiple_of(t0 + B_CHUNK, B_CHUNK)
        tp = pl.multiple_of(jnp.maximum(t0 - B_CHUNK, 0), B_CHUNK)
        b_project(t0, buf_a, buf_b, c == 0)
        b_attend(tp, buf_b)
        b_project(t1, buf_b, buf_a, None)
        b_attend(t0, buf_a)
        for j in range(3):
            cp_w(c, j).wait()
        for i in range(ppc):
            prepare_pair(c * ppc + i)
        return carry

    lax.fori_loop(0, n_chunk, b_body, 0)
    cp_bwo.wait()
    for s in range(n_slab):
        slab[s, 0:D, :] = bwo_v[:, s * LANES:(s + 1) * LANES].astype(F32)
        for d in range(bdh):
            bwo_p[d * B_HEADS:(d + 1) * B_HEADS, s * LANES:(s + 1) * LANES] = slab[
                s, pl.ds(d, B_HEADS, stride=bdh), :].astype(BF16)
    b_attend(S - B_CHUNK, buf_b)
    b_v[...] = _dot(ob_v[0:seg, :], bwo_p[...])
    cp_wo.wait()

    scale = dh ** -0.5

    def step(s, mem):
        r0 = pl.multiple_of(s * seg, seg)
        h = jnp.concatenate([mem, x_v[pl.ds(r0, seg), :].astype(F32)], axis=0)

        row = lax.broadcasted_iota(jnp.int32, (L, 2 * L), 0)
        col = lax.broadcasted_iota(jnp.int32, (L, 2 * L), 1)
        first = col < L
        visible = (row < M) | (row >= jnp.where(first, col, col - L))
        lo = lax.broadcasted_iota(jnp.int32, (L, PW), 1) < dh

        def block_diag(t):
            return jnp.concatenate(
                [jnp.where(lo, t, 0.0), jnp.where(lo, 0.0, t)],
                axis=0).astype(BF16)

        def project(p):
            q = jnp.concatenate(
                [_dot(h[:L - PRE], w_v[p, :, :PW]),
                 qpre[p, pl.ds(pl.multiple_of(s * PRE, PRE), PRE), :]], axis=0)
            kv = _dot(h, w_v[p, :, PW:])
            return q, block_diag(kv[:, :PW]), block_diag(kv[:, PW:])

        def scores(q, kb):
            sc = jnp.where(visible, _dot_nt(q, kb) * scale, NEG)
            ma = jnp.max(jnp.where(first, sc, -jnp.inf), axis=-1, keepdims=True)
            mb = jnp.max(jnp.where(first, -jnp.inf, sc), axis=-1, keepdims=True)
            e = jnp.exp(sc - jnp.where(first, ma, mb))
            sa = jnp.sum(jnp.where(first, e, 0.0), axis=-1, keepdims=True)
            sb = jnp.sum(jnp.where(first, 0.0, e), axis=-1, keepdims=True)
            return e * jnp.where(first, 1.0 / sa, 1.0 / sb)

        proj, prob, outs = {}, {}, {}
        acc = None

        def out_proj(acc, pairs):
            for p in pairs:
                y = _dot(outs[p], wo_v[p * PW:(p + 1) * PW, :])
                acc = y if acc is None else acc + y
            return acc

        for t in range(n_pair + 2):
            if t < n_pair:
                proj[t] = project(t)
            if t == n_pair:
                acc = out_proj(acc, range(0, n_pair // 4))
            if 0 <= t - 1 < n_pair:
                prob[t - 1] = scores(proj[t - 1][0], proj[t - 1][1])
            if t == n_pair + 1:
                acc = out_proj(acc, range(n_pair // 4, n_pair - 4))
            if 0 <= t - 2 < n_pair:
                outs[t - 2] = _dot(prob[t - 2], proj[t - 2][2])
        acc = out_proj(acc, range(n_pair - 4, n_pair))

        g = g_v[pl.ds(r0, seg), :]
        g = jnp.concatenate([g] * n_slab, axis=1)
        out_v[pl.ds(r0, seg), :] = (
            g * acc[M:] + (1.0 - g) * b_v[...]).astype(out_v.dtype)
        r1 = pl.multiple_of(jnp.minimum(r0 + seg, S - seg), seg)
        b_v[...] = _dot(ob_v[pl.ds(r1, seg), :], bwo_p[...])
        pltpu.make_async_copy(out_v.at[pl.ds(r0, seg)],
                              out_hbm.at[pl.ds(r0, seg)], sem_out.at[0]).start()
        return acc[:M]

    lax.fori_loop(0, n_seg, step, mem0_ref[...].astype(F32), unroll=UNROLL)
    pltpu.make_async_copy(out_v, out_v, sem_out.at[0]).wait()


@functools.partial(jax.jit, static_argnames=("A_seg_len",))
def pallas_gated_mix__memory_aug_recurrent_mem_tr__sliding_local_dilated__prompt_kernel(
    A_x: jax.Array,
    A_mem0: jax.Array,
    A_Wq: jax.Array,
    A_Wk: jax.Array,
    A_Wv: jax.Array,
    A_Wo: jax.Array,
    A_seg_len: int,
    B_x: jax.Array,
    B_wqkv: jax.Array,
    B_wo: jax.Array,
    gate_w: jax.Array,
):
    del B_x
    _, S, D = A_x.shape
    _, H, Dh = A_Wq.shape
    M = A_mem0.shape[1]
    seg = int(A_seg_len)
    n_pair = H // 2
    n_slab = D // LANES
    n_chunk = S // (2 * B_CHUNK)

    def by_head(w):
        return jnp.transpose(w, (1, 2, 0)).reshape(H * Dh, D)

    qkv_buf = [pltpu.VMEM((n_slab, B_CHUNK, LANES), F32),
               pltpu.VMEM((n_slab, B_CHUNK + B_PAD, LANES), F32),
               pltpu.VMEM((n_slab, B_CHUNK + B_PAD, LANES), F32)]
    hbm = pl.BlockSpec(memory_space=pl.ANY)
    vmem = pl.BlockSpec(memory_space=pltpu.VMEM)
    out = pl.pallas_call(
        functools.partial(_kernel, seg=seg, n_heads=H, dh=Dh),
        out_shape=jax.ShapeDtypeStruct((S, D), A_x.dtype),
        in_specs=[hbm, vmem, hbm, hbm, hbm, hbm, hbm, hbm, vmem],
        out_specs=hbm,
        scratch_shapes=[
            pltpu.VMEM((S, D), BF16),
            pltpu.VMEM((S // seg * PRE, D), BF16),
            pltpu.VMEM((3, H * Dh, D), BF16),
            pltpu.VMEM((n_pair, D, 6 * Dh), BF16),
            pltpu.VMEM((H * Dh, D), BF16),
            pltpu.VMEM((D, 3 * D), BF16),
            pltpu.VMEM((D, D), BF16),
            pltpu.VMEM((n_slab, 3 * D, LANES), F32),
            pltpu.VMEM((3 * D, D), BF16),
            pltpu.VMEM((D, D), BF16),
            *qkv_buf, *qkv_buf,
            pltpu.VMEM((S, LANES), F32),
            pltpu.VMEM((S, D), BF16),
            pltpu.VMEM((seg, D), F32),
            pltpu.VMEM((n_pair, S // seg * PRE, 2 * Dh), F32),
            pltpu.VMEM((S, D), A_x.dtype),
            pltpu.SemaphoreType.DMA((3,)),
            pltpu.SemaphoreType.DMA((n_slab,)),
            pltpu.SemaphoreType.DMA((n_chunk, 3)),
            pltpu.SemaphoreType.DMA((1,)),
        ],
        compiler_params=pltpu.CompilerParams(
            vmem_limit_bytes=110 * 1024 * 1024),
    )(A_x.reshape(S, D), A_mem0.reshape(M, D), by_head(A_Wq), by_head(A_Wk),
      by_head(A_Wv), A_Wo.reshape(H * Dh, D), B_wqkv, B_wo,
      gate_w.reshape(1, D))
    return out.reshape(1, S, D)
```

```python
import functools

import jax
import jax.numpy as jnp
from jax import lax
import jax.experimental.pallas as pl
import jax.experimental.pallas.tpu as pltpu

F32 = jnp.float32
BF16 = jnp.bfloat16
LANES = 128
NEG = -1000000000.0

B_HEADS = 32
B_WIN = 8
B_DIL = 2
B_PAD = 16
B_CHUNK = 128
PRE = 8
UNROLL = 2
B_SUB = 32


def _dot(a, b):
    return lax.dot_general(a, b, (((1,), (0,)), ((), ())),
                           preferred_element_type=F32)


def _dot_nt(a, b):
    return lax.dot_general(a, b, (((1,), (1,)), ((), ())),
                           preferred_element_type=F32)


def _interleave(*stages):
    stages = list(stages)
    while stages:
        for g in list(stages):
            if next(g, _DONE) is _DONE:
                stages.remove(g)


_DONE = object()


def _kernel(x_hbm, mem0_ref, wq_hbm, wk_hbm, wv_hbm, wo_hbm, bqkv_hbm, bwo_hbm,
            gate_ref, out_hbm,
            x_v, xt_v, wraw, w_v, wo_v, bqkv_v, bwo_v, slab, bqkv_p, bwo_p,
            q_a, k_a, v_a, q_b, k_b, v_b, g_v, ob_v, qpre, out_v,
            sem_in, sem_b, sem_w, sem_out,
            *, seg, n_heads, dh):
    S, D = x_v.shape
    M = mem0_ref.shape[0]
    L = M + seg
    n_seg = S // seg
    n_pair = n_heads // 2
    PW = 2 * dh
    n_slab = D // LANES
    bdh = D // B_HEADS
    n_chunk = S // (2 * B_CHUNK)
    ppc = n_pair // n_chunk
    buf_a, buf_b = (q_a, k_a, v_a), (q_b, k_b, v_b)

    x_head = 4 * B_CHUNK
    cp_x0 = pltpu.make_async_copy(x_hbm.at[0:x_head], x_v.at[0:x_head],
                                  sem_in.at[0])
    cp_x1 = pltpu.make_async_copy(x_hbm.at[x_head:S], x_v.at[x_head:S],
                                  sem_in.at[1])
    cp_bwo = pltpu.make_async_copy(bwo_hbm, bwo_v, sem_in.at[2])

    def cp_bqkv(s):
        rows = pl.ds(s * LANES, LANES)
        return pltpu.make_async_copy(bqkv_hbm.at[rows], bqkv_v.at[rows],
                                     sem_b.at[s])

    def cp_w(c, j):
        rows = pl.ds(pl.multiple_of(c * ppc * PW, PW), ppc * PW)
        src = (wq_hbm, wk_hbm, wv_hbm, wo_hbm)[j]
        dst = wo_v.at[rows] if j == 3 else wraw.at[j, rows]
        return pltpu.make_async_copy(src.at[rows], dst, sem_w.at[c, j])

    for s in range(n_slab):
        cp_bqkv(s).start()
    cp_x0.start()
    for ref in buf_b:
        ref[...] = jnp.zeros(ref.shape, ref.dtype)

    for s in range(n_slab):
        cp_bqkv(s).wait()
        if s == n_slab - 1:
            cp_x1.start()
            for j in range(3):
                cp_w(0, j).start()
        slab[s] = bqkv_v[s * LANES:(s + 1) * LANES, :].astype(F32).T
        for part in range(3):
            for d in range(bdh):
                r0 = part * D + d * B_HEADS
                bqkv_p[r0:r0 + B_HEADS, s * LANES:(s + 1) * LANES] = slab[
                    s, pl.ds(part * D + d, B_HEADS, stride=bdh), :].astype(BF16)
    cp_x0.wait()

    bscale = bdh ** -0.5
    gate = gate_ref[...].astype(F32)

    def b_project(t0, dst, prev, is_first):
        for j in range(3):
            y = _dot_nt(x_v[pl.ds(t0, B_CHUNK), :], bqkv_p[j * D:(j + 1) * D, :])
            for s in range(n_slab):
                t = y[:, s * LANES:(s + 1) * LANES]
                if j == 0:
                    dst[j][s] = t
                    continue
                halo = prev[j][s, B_CHUNK:, :]
                if is_first is not None:
                    halo = jnp.where(
                        is_first, jnp.broadcast_to(t[0:1], halo.shape), halo)
                dst[j][s, 0:B_PAD, :] = halo
                dst[j][s, B_PAD:, :] = t
            yield

    def b_attend(t0, src):
        q_s, k_s, v_s = src
        for r in range(0, B_CHUNK, B_SUB):
            qs = [q_s[s, r:r + B_SUB, :] for s in range(n_slab)]
            logits = []
            for w in range(B_WIN):
                o = B_PAD + r - w * B_DIL
                acc = qs[0] * k_s[0, o:o + B_SUB, :]
                for s in range(1, n_slab):
                    acc = acc + qs[s] * k_s[s, o:o + B_SUB, :]
                acc = acc + pltpu.roll(acc, 64, 1)
                acc = acc + pltpu.roll(acc, 32, 1)
                acc = acc * bscale
                if r < w * B_DIL:
                    pos = t0 + r + lax.broadcasted_iota(
                        jnp.int32, (B_SUB, LANES), 0)
                    acc = jnp.where(pos >= w * B_DIL, acc, NEG)
                logits.append(acc)
            mx = functools.reduce(jnp.maximum, logits)
            es = [jnp.exp(l - mx) for l in logits]
            inv = 1.0 / functools.reduce(jnp.add, es)
            cols = []
            for s in range(n_slab):
                acc = None
                for w in range(B_WIN):
                    o = B_PAD + r - w * B_DIL
                    t = es[w] * v_s[s, o:o + B_SUB, :]
                    acc = t if acc is None else acc + t
                cols.append((acc * inv).astype(BF16))
            rows = pl.ds(t0 + r, B_SUB)
            ob_v[rows, :] = jnp.concatenate(cols, axis=1)
            g = jax.nn.sigmoid(jnp.sum(x_v[rows, :].astype(F32) * gate,
                                       axis=-1, keepdims=True))
            g_v[rows, :] = jnp.broadcast_to(g, (B_SUB, LANES))
            if (r // B_SUB) % 2:
                yield

    def prepare(c):
        for i in range(ppc):
            p = c * ppc + i
            rows = pl.ds(pl.multiple_of(p * PW, PW), PW)
            qpre[p] = _dot_nt(xt_v[...], wraw[0, rows, :])
            yield
            for j in range(3):
                w_v[p, :, j * PW:(j + 1) * PW] = wraw[j, rows, :].T
            yield

    def b_body(c, carry):
        t0 = pl.multiple_of(c * 2 * B_CHUNK, B_CHUNK)
        t1 = pl.multiple_of(t0 + B_CHUNK, B_CHUNK)
        tp = pl.multiple_of(jnp.maximum(t0 - B_CHUNK, 0), B_CHUNK)
        _interleave(b_project(t0, buf_a, buf_b, c == 0), b_attend(tp, buf_b))
        _interleave(b_project(t1, buf_b, buf_a, None), b_attend(t0, buf_a))

        @pl.when(c == 1)
        def _():
            cp_x1.wait()
            for i in range(0, n_seg, 2):
                xt_v[i * PRE:(i + 2) * PRE, :] = jnp.concatenate(
                    [x_v[(i + u + 1) * seg - 2 * PRE:(i + u + 1) * seg, :]
                     .astype(F32)[PRE:] for u in range(2)], axis=0).astype(BF16)

        @pl.when(c > 0)
        def _():
            for j in range(3):
                cp_w(c - 1, j).wait()

        @pl.when(c + 1 < n_chunk)
        def _():
            for j in range(3):
                cp_w(c + 1, j).start()

        cp_w(c, 3).start()

        @pl.when(c == n_chunk - 1)
        def _():
            cp_bwo.start()

        @pl.when(c > 0)
        def _():
            _interleave(prepare(c - 1))
        return carry

    lax.fori_loop(0, n_chunk, b_body, 0)

    def permute_bwo():
        for s in range(n_slab):
            slab[s, 0:D, :] = bwo_v[:, s * LANES:(s + 1) * LANES].astype(F32)
            for d in range(bdh):
                bwo_p[d * B_HEADS:(d + 1) * B_HEADS,
                      s * LANES:(s + 1) * LANES] = slab[
                    s, pl.ds(d, B_HEADS, stride=bdh), :].astype(BF16)
        yield

    cp_bwo.wait()
    for j in range(3):
        cp_w(n_chunk - 1, j).wait()
    _interleave(prepare(n_chunk - 1), permute_bwo(),
                b_attend(S - B_CHUNK, buf_b))
    for c in range(n_chunk):
        cp_w(c, 3).wait()

    scale = dh ** -0.5

    def step(s, mem):
        r0 = pl.multiple_of(s * seg, seg)
        h = jnp.concatenate([mem, x_v[pl.ds(r0, seg), :].astype(F32)], axis=0)

        row = lax.broadcasted_iota(jnp.int32, (L, 2 * L), 0)
        col = lax.broadcasted_iota(jnp.int32, (L, 2 * L), 1)
        first = col < L
        visible = (row < M) | (row >= jnp.where(first, col, col - L))
        lo = lax.broadcasted_iota(jnp.int32, (L, PW), 1) < dh

        def block_diag(t):
            return jnp.concatenate(
                [jnp.where(lo, t, 0.0), jnp.where(lo, 0.0, t)],
                axis=0).astype(BF16)

        def project(p):
            q = jnp.concatenate(
                [_dot(h[:L - PRE], w_v[p, :, :PW]),
                 qpre[p, pl.ds(pl.multiple_of(s * PRE, PRE), PRE), :]], axis=0)
            kv = _dot(h, w_v[p, :, PW:])
            return q, block_diag(kv[:, :PW]), block_diag(kv[:, PW:])

        def scores(q, kb):
            sc = jnp.where(visible, _dot_nt(q, kb) * scale, NEG)
            ma = jnp.max(jnp.where(first, sc, -jnp.inf), axis=-1, keepdims=True)
            mb = jnp.max(jnp.where(first, -jnp.inf, sc), axis=-1, keepdims=True)
            e = jnp.exp(sc - jnp.where(first, ma, mb))
            sa = jnp.sum(jnp.where(first, e, 0.0), axis=-1, keepdims=True)
            sb = jnp.sum(jnp.where(first, 0.0, e), axis=-1, keepdims=True)
            return e * jnp.where(first, 1.0 / sa, 1.0 / sb)

        proj, prob, outs = {}, {}, {}
        acc = None

        def out_proj(acc, pairs):
            for p in pairs:
                y = _dot(outs[p], wo_v[p * PW:(p + 1) * PW, :])
                acc = y if acc is None else acc + y
            return acc

        for t in range(n_pair + 2):
            if t < n_pair:
                proj[t] = project(t)
            if t == n_pair:
                acc = out_proj(acc, range(0, n_pair // 4))
            if 0 <= t - 1 < n_pair:
                prob[t - 1] = scores(proj[t - 1][0], proj[t - 1][1])
            if t == n_pair + 1:
                acc = out_proj(acc, range(n_pair // 4, n_pair - 4))
            if 0 <= t - 2 < n_pair:
                outs[t - 2] = _dot(prob[t - 2], proj[t - 2][2])
        acc = out_proj(acc, range(n_pair - 4, n_pair))

        b = _dot(ob_v[pl.ds(r0, seg), :], bwo_p[...])
        g = g_v[pl.ds(r0, seg), :]
        g = jnp.concatenate([g] * n_slab, axis=1)
        out_v[pl.ds(r0, seg), :] = (
            g * acc[M:] + (1.0 - g) * b).astype(out_v.dtype)
        pltpu.make_async_copy(out_v.at[pl.ds(r0, seg)],
                              out_hbm.at[pl.ds(r0, seg)], sem_out.at[0]).start()
        return acc[:M]

    lax.fori_loop(0, n_seg, step, mem0_ref[...].astype(F32), unroll=UNROLL)
    pltpu.make_async_copy(out_v, out_v, sem_out.at[0]).wait()


@functools.partial(jax.jit, static_argnames=("A_seg_len",))
def pallas_gated_mix__memory_aug_recurrent_mem_tr__sliding_local_dilated__prompt_kernel(
    A_x: jax.Array,
    A_mem0: jax.Array,
    A_Wq: jax.Array,
    A_Wk: jax.Array,
    A_Wv: jax.Array,
    A_Wo: jax.Array,
    A_seg_len: int,
    B_x: jax.Array,
    B_wqkv: jax.Array,
    B_wo: jax.Array,
    gate_w: jax.Array,
):
    del B_x
    _, S, D = A_x.shape
    _, H, Dh = A_Wq.shape
    M = A_mem0.shape[1]
    seg = int(A_seg_len)
    n_pair = H // 2
    n_slab = D // LANES
    n_chunk = S // (2 * B_CHUNK)

    def by_head(w):
        return jnp.transpose(w, (1, 2, 0)).reshape(H * Dh, D)

    qkv_buf = [pltpu.VMEM((n_slab, B_CHUNK, LANES), F32),
               pltpu.VMEM((n_slab, B_CHUNK + B_PAD, LANES), F32),
               pltpu.VMEM((n_slab, B_CHUNK + B_PAD, LANES), F32)]
    hbm = pl.BlockSpec(memory_space=pl.ANY)
    vmem = pl.BlockSpec(memory_space=pltpu.VMEM)
    out = pl.pallas_call(
        functools.partial(_kernel, seg=seg, n_heads=H, dh=Dh),
        out_shape=jax.ShapeDtypeStruct((S, D), A_x.dtype),
        in_specs=[hbm, vmem, hbm, hbm, hbm, hbm, hbm, hbm, vmem],
        out_specs=hbm,
        scratch_shapes=[
            pltpu.VMEM((S, D), BF16),
            pltpu.VMEM((S // seg * PRE, D), BF16),
            pltpu.VMEM((3, H * Dh, D), BF16),
            pltpu.VMEM((n_pair, D, 6 * Dh), BF16),
            pltpu.VMEM((H * Dh, D), BF16),
            pltpu.VMEM((D, 3 * D), BF16),
            pltpu.VMEM((D, D), BF16),
            pltpu.VMEM((n_slab, 3 * D, LANES), F32),
            pltpu.VMEM((3 * D, D), BF16),
            pltpu.VMEM((D, D), BF16),
            *qkv_buf, *qkv_buf,
            pltpu.VMEM((S, LANES), F32),
            pltpu.VMEM((S, D), BF16),
            pltpu.VMEM((n_pair, S // seg * PRE, 2 * Dh), F32),
            pltpu.VMEM((S, D), A_x.dtype),
            pltpu.SemaphoreType.DMA((3,)),
            pltpu.SemaphoreType.DMA((n_slab,)),
            pltpu.SemaphoreType.DMA((n_chunk, 4)),
            pltpu.SemaphoreType.DMA((1,)),
        ],
        compiler_params=pltpu.CompilerParams(
            vmem_limit_bytes=110 * 1024 * 1024),
    )(A_x.reshape(S, D), A_mem0.reshape(M, D), by_head(A_Wq), by_head(A_Wk),
      by_head(A_Wv), A_Wo.reshape(H * Dh, D), B_wqkv, B_wo,
      gate_w.reshape(1, D))
    return out.reshape(1, S, D)
```

```python
import functools

import jax
import jax.numpy as jnp
from jax import lax
import jax.experimental.pallas as pl
import jax.experimental.pallas.tpu as pltpu

F32 = jnp.float32
BF16 = jnp.bfloat16
LANES = 128
NEG = -1000000000.0

B_HEADS = 32
B_WIN = 8
B_DIL = 2
B_PAD = 16
B_CHUNK = 128
PRE = 8
UNROLL = 4
B_SUB = 32


def _dot(a, b):
    return lax.dot_general(a, b, (((1,), (0,)), ((), ())),
                           preferred_element_type=F32)


def _dot_nt(a, b):
    return lax.dot_general(a, b, (((1,), (1,)), ((), ())),
                           preferred_element_type=F32)


def _interleave(*stages):
    stages = list(stages)
    while stages:
        for g in list(stages):
            if next(g, _DONE) is _DONE:
                stages.remove(g)


_DONE = object()


def _kernel(x_hbm, mem0_ref, wq_hbm, wk_hbm, wv_hbm, wo_hbm, bqkv_hbm, bwo_hbm,
            gate_ref, out_hbm,
            x_v, xt_v, wraw, w_v, wo_v, bqkv_v, bwo_v, slab, bqkv_p, bwo_p,
            q_a, k_a, v_a, q_b, k_b, v_b, g_v, ob_v, qpre, out_v,
            sem_in, sem_b, sem_w, sem_out,
            *, seg, n_heads, dh):
    S, D = x_v.shape
    M = mem0_ref.shape[0]
    L = M + seg
    n_seg = S // seg
    n_pair = n_heads // 2
    PW = 2 * dh
    n_slab = D // LANES
    bdh = D // B_HEADS
    n_chunk = S // (2 * B_CHUNK)
    ppc = n_pair // n_chunk
    buf_a, buf_b = (q_a, k_a, v_a), (q_b, k_b, v_b)

    x_head = 4 * B_CHUNK
    cp_x0 = pltpu.make_async_copy(x_hbm.at[0:x_head], x_v.at[0:x_head],
                                  sem_in.at[0])
    cp_x1 = pltpu.make_async_copy(x_hbm.at[x_head:S], x_v.at[x_head:S],
                                  sem_in.at[1])
    cp_bwo = pltpu.make_async_copy(bwo_hbm, bwo_v, sem_in.at[2])

    def cp_bqkv(s):
        rows = pl.ds(s * LANES, LANES)
        return pltpu.make_async_copy(bqkv_hbm.at[rows], bqkv_v.at[rows],
                                     sem_b.at[s])

    def cp_w(c, j):
        rows = pl.ds(pl.multiple_of(c * ppc * PW, PW), ppc * PW)
        src = (wq_hbm, wk_hbm, wv_hbm, wo_hbm)[j]
        dst = wo_v.at[rows] if j == 3 else wraw.at[j, rows]
        return pltpu.make_async_copy(src.at[rows], dst, sem_w.at[c, j])

    for s in range(n_slab):
        cp_bqkv(s).start()
    cp_x0.start()
    for ref in buf_b:
        ref[...] = jnp.zeros(ref.shape, ref.dtype)

    for s in range(n_slab):
        cp_bqkv(s).wait()
        if s == n_slab - 1:
            cp_x1.start()
            for j in range(3):
                cp_w(0, j).start()
        slab[s, 0:3 * D, :] = bqkv_v[s * LANES:(s + 1) * LANES, :].astype(F32).T
        for part in range(3):
            for d in range(bdh):
                r0 = part * D + d * B_HEADS
                bqkv_p[r0:r0 + B_HEADS, s * LANES:(s + 1) * LANES] = slab[
                    s, pl.ds(part * D + d, B_HEADS, stride=bdh), :].astype(BF16)
    cp_x0.wait()

    bscale = bdh ** -0.5
    gate = gate_ref[...].astype(F32).reshape(1, D)

    def b_project(t0, dst, prev, is_first):
        for j in range(3):
            y = _dot_nt(x_v[pl.ds(t0, B_CHUNK), :], bqkv_p[j * D:(j + 1) * D, :])
            for s in range(n_slab):
                t = y[:, s * LANES:(s + 1) * LANES]
                if j == 0:
                    dst[j][s] = t
                    continue
                halo = prev[j][s, B_CHUNK:, :]
                if is_first is not None:
                    halo = jnp.where(
                        is_first, jnp.broadcast_to(t[0:1], halo.shape), halo)
                dst[j][s, 0:B_PAD, :] = halo
                dst[j][s, B_PAD:, :] = t
            yield

    def b_attend(t0, src):
        q_s, k_s, v_s = src
        for r in range(0, B_CHUNK, B_SUB):
            qs = [q_s[s, r:r + B_SUB, :] for s in range(n_slab)]
            logits = []
            for w in range(B_WIN):
                o = B_PAD + r - w * B_DIL
                acc = qs[0] * k_s[0, o:o + B_SUB, :]
                for s in range(1, n_slab):
                    acc = acc + qs[s] * k_s[s, o:o + B_SUB, :]
                acc = acc + pltpu.roll(acc, 64, 1)
                acc = acc + pltpu.roll(acc, 32, 1)
                acc = acc * bscale
                if r < w * B_DIL:
                    pos = t0 + r + lax.broadcasted_iota(
                        jnp.int32, (B_SUB, LANES), 0)
                    acc = jnp.where(pos >= w * B_DIL, acc, NEG)
                logits.append(acc)
            mx = functools.reduce(jnp.maximum, logits)
            es = [jnp.exp(l - mx) for l in logits]
            inv = 1.0 / functools.reduce(jnp.add, es)
            cols = []
            for s in range(n_slab):
                acc = None
                for w in range(B_WIN):
                    o = B_PAD + r - w * B_DIL
                    t = es[w] * v_s[s, o:o + B_SUB, :]
                    acc = t if acc is None else acc + t
                cols.append((acc * inv).astype(BF16))
            rows = pl.ds(t0 + r, B_SUB)
            ob_v[rows, :] = jnp.concatenate(cols, axis=1)
            g = jax.nn.sigmoid(jnp.sum(x_v[rows, :].astype(F32) * gate,
                                       axis=-1, keepdims=True))
            g_v[rows, :] = jnp.broadcast_to(g, (B_SUB, LANES))
            if (r // B_SUB) % 2:
                yield

    def prepare(c):
        for i in range(ppc):
            p = c * ppc + i
            rows = pl.ds(pl.multiple_of(p * PW, PW), PW)
            qpre[p] = _dot_nt(xt_v[...], wraw[0, rows, :])
            yield
            for j in range(3):
                w_v[p, :, j * PW:(j + 1) * PW] = wraw[j, rows, :].T
            yield

    def b_body(c, carry):
        t0 = pl.multiple_of(c * 2 * B_CHUNK, B_CHUNK)
        t1 = pl.multiple_of(t0 + B_CHUNK, B_CHUNK)
        tp = pl.multiple_of(jnp.maximum(t0 - B_CHUNK, 0), B_CHUNK)
        _interleave(b_project(t0, buf_a, buf_b, c == 0), b_attend(tp, buf_b))
        _interleave(b_project(t1, buf_b, buf_a, None), b_attend(t0, buf_a))

        @pl.when(c == 1)
        def _():
            cp_x1.wait()
            for i in range(0, n_seg, 2):
                xt_v[i * PRE:(i + 2) * PRE, :] = jnp.concatenate(
                    [x_v[(i + u + 1) * seg - 2 * PRE:(i + u + 1) * seg, :]
                     .astype(F32)[PRE:] for u in range(2)], axis=0).astype(BF16)

        @pl.when(c > 0)
        def _():
            for j in range(3):
                cp_w(c - 1, j).wait()

        @pl.when(c + 1 < n_chunk)
        def _():
            for j in range(3):
                cp_w(c + 1, j).start()

        cp_w(c, 3).start()

        @pl.when(c == n_chunk - 1)
        def _():
            cp_bwo.start()

        @pl.when(c > 0)
        def _():
            _interleave(prepare(c - 1))
        return carry

    lax.fori_loop(0, n_chunk, b_body, 0)

    def permute_bwo():
        for s in range(n_slab):
            slab[s, 0:D, :] = bwo_v[:, s * LANES:(s + 1) * LANES].astype(F32)
            for d in range(bdh):
                bwo_p[d * B_HEADS:(d + 1) * B_HEADS,
                      s * LANES:(s + 1) * LANES] = slab[
                    s, pl.ds(d, B_HEADS, stride=bdh), :].astype(BF16)
        yield

    cp_bwo.wait()
    for j in range(3):
        cp_w(n_chunk - 1, j).wait()
    _interleave(prepare(n_chunk - 1), permute_bwo(),
                b_attend(S - B_CHUNK, buf_b))
    for c in range(n_chunk):
        cp_w(c, 3).wait()

    scale = dh ** -0.5

    def step(s, mem):
        r0 = pl.multiple_of(s * seg, seg)
        h = jnp.concatenate([mem, x_v[pl.ds(r0, seg), :].astype(F32)], axis=0)

        row = lax.broadcasted_iota(jnp.int32, (L, 2 * L), 0)
        col = lax.broadcasted_iota(jnp.int32, (L, 2 * L), 1)
        first = col < L
        visible = (row < M) | (row >= jnp.where(first, col, col - L))
        lo = lax.broadcasted_iota(jnp.int32, (L, PW), 1) < dh

        def block_diag(t):
            return jnp.concatenate(
                [jnp.where(lo, t, 0.0), jnp.where(lo, 0.0, t)],
                axis=0).astype(BF16)

        def project(p):
            q = jnp.concatenate(
                [_dot(h[:L - PRE], w_v[p, :, :PW]),
                 qpre[p, pl.ds(pl.multiple_of(s * PRE, PRE), PRE), :]], axis=0)
            kv = _dot(h, w_v[p, :, PW:])
            return q, block_diag(kv[:, :PW]), block_diag(kv[:, PW:])

        def scores(q, kb):
            sc = jnp.where(visible, _dot_nt(q, kb) * scale, NEG)
            ma = jnp.max(jnp.where(first, sc, -jnp.inf), axis=-1, keepdims=True)
            mb = jnp.max(jnp.where(first, -jnp.inf, sc), axis=-1, keepdims=True)
            e = jnp.exp(sc - jnp.where(first, ma, mb))
            sa = jnp.sum(jnp.where(first, e, 0.0), axis=-1, keepdims=True)
            sb = jnp.sum(jnp.where(first, 0.0, e), axis=-1, keepdims=True)
            return e * jnp.where(first, 1.0 / sa, 1.0 / sb)

        proj, prob, outs = {}, {}, {}
        acc = None

        def out_proj(acc, pairs):
            for p in pairs:
                y = _dot(outs[p], wo_v[p * PW:(p + 1) * PW, :])
                acc = y if acc is None else acc + y
            return acc

        for t in range(n_pair + 2):
            if t < n_pair:
                proj[t] = project(t)
            if t == n_pair:
                acc = out_proj(acc, range(0, n_pair // 4))
            if 0 <= t - 1 < n_pair:
                prob[t - 1] = scores(proj[t - 1][0], proj[t - 1][1])
            if t == n_pair + 1:
                acc = out_proj(acc, range(n_pair // 4, n_pair - 4))
            if 0 <= t - 2 < n_pair:
                outs[t - 2] = _dot(prob[t - 2], proj[t - 2][2])
        acc = out_proj(acc, range(n_pair - 4, n_pair))

        b = _dot(ob_v[pl.ds(r0, seg), :], bwo_p[...])
        g = g_v[pl.ds(r0, seg), :]
        g = jnp.concatenate([g] * n_slab, axis=1)
        out_v[pl.ds(r0, seg), :] = (
            g * acc[M:] + (1.0 - g) * b).astype(out_v.dtype)
        pltpu.make_async_copy(out_v.at[pl.ds(r0, seg)],
                              out_hbm.at[pl.ds(r0, seg)], sem_out.at[0]).start()
        return acc[:M]

    lax.fori_loop(0, n_seg, step, mem0_ref[...].astype(F32), unroll=UNROLL)
    pltpu.make_async_copy(out_v, out_v, sem_out.at[0]).wait()


@functools.partial(jax.jit, static_argnames=("A_seg_len",))
def pallas_gated_mix__memory_aug_recurrent_mem_tr__sliding_local_dilated__prompt_kernel(
    A_x: jax.Array,
    A_mem0: jax.Array,
    A_Wq: jax.Array,
    A_Wk: jax.Array,
    A_Wv: jax.Array,
    A_Wo: jax.Array,
    A_seg_len: int,
    B_x: jax.Array,
    B_wqkv: jax.Array,
    B_wo: jax.Array,
    gate_w: jax.Array,
):
    del B_x
    _, S, D = A_x.shape
    _, H, Dh = A_Wq.shape
    M = A_mem0.shape[1]
    seg = int(A_seg_len)
    n_pair = H // 2
    n_slab = D // LANES
    n_chunk = S // (2 * B_CHUNK)

    def by_head(w):
        return jnp.transpose(w, (1, 2, 0)).reshape(H * Dh, D)

    qkv_buf = [pltpu.VMEM((n_slab, B_CHUNK, LANES), F32),
               pltpu.VMEM((n_slab, B_CHUNK + B_PAD, LANES), F32),
               pltpu.VMEM((n_slab, B_CHUNK + B_PAD, LANES), F32)]
    hbm = pl.BlockSpec(memory_space=pl.ANY)
    vmem = pl.BlockSpec(memory_space=pltpu.VMEM)
    out = pl.pallas_call(
        functools.partial(_kernel, seg=seg, n_heads=H, dh=Dh),
        out_shape=jax.ShapeDtypeStruct((S, D), A_x.dtype),
        in_specs=[hbm, vmem, hbm, hbm, hbm, hbm, hbm, hbm, vmem],
        out_specs=hbm,
        scratch_shapes=[
            pltpu.VMEM((S, D), BF16),
            pltpu.VMEM((S // seg * PRE, D), BF16),
            pltpu.VMEM((3, H * Dh, D), BF16),
            pltpu.VMEM((n_pair, D, 6 * Dh), BF16),
            pltpu.VMEM((H * Dh, D), BF16),
            pltpu.VMEM((D, 3 * D), BF16),
            pltpu.VMEM((D, D), BF16),
            pltpu.VMEM((n_slab, 3 * D + B_HEADS, LANES), F32),
            pltpu.VMEM((3 * D, D), BF16),
            pltpu.VMEM((D, D), BF16),
            *qkv_buf, *qkv_buf,
            pltpu.VMEM((S, LANES), F32),
            pltpu.VMEM((S, D), BF16),
            pltpu.VMEM((n_pair, S // seg * PRE, 2 * Dh), F32),
            pltpu.VMEM((S, D), A_x.dtype),
            pltpu.SemaphoreType.DMA((3,)),
            pltpu.SemaphoreType.DMA((n_slab,)),
            pltpu.SemaphoreType.DMA((n_chunk, 4)),
            pltpu.SemaphoreType.DMA((1,)),
        ],
        compiler_params=pltpu.CompilerParams(
            vmem_limit_bytes=110 * 1024 * 1024),
    )(A_x.reshape(S, D), A_mem0.reshape(M, D), by_head(A_Wq), by_head(A_Wk),
      by_head(A_Wv), A_Wo.reshape(H * Dh, D), B_wqkv, B_wo,
      gate_w)
    return out.reshape(1, S, D)
```

```python
import functools

import jax
import jax.numpy as jnp
from jax import lax
import jax.experimental.pallas as pl
import jax.experimental.pallas.tpu as pltpu

F32 = jnp.float32
BF16 = jnp.bfloat16
LANES = 128
NEG = -1000000000.0
LOG2E = 1.4426950408889634

B_HEADS = 32
B_WIN = 8
B_DIL = 2
B_PAD = 16
B_CHUNK = 128
PRE = 8
UNROLL = 4
B_SUB = 32


def _dot(a, b):
    return lax.dot_general(a, b, (((1,), (0,)), ((), ())),
                           preferred_element_type=F32)


def _dot_nt(a, b):
    return lax.dot_general(a, b, (((1,), (1,)), ((), ())),
                           preferred_element_type=F32)


def _interleave(*stages):
    stages = list(stages)
    while stages:
        for g in list(stages):
            if next(g, _DONE) is _DONE:
                stages.remove(g)


_DONE = object()


def _kernel(x_hbm, mem0_ref, wq_hbm, wk_hbm, wv_hbm, wo_hbm, bqkv_hbm, bwo_hbm,
            gate_ref, out_hbm,
            x_v, xt_v, wraw, w_v, wo_v, bqkv_v, bwo_v, slab, bqkv_p, bwo_p,
            q_a, k_a, v_a, q_b, k_b, v_b, g_v, ob_v, qpre, out_v,
            sem_in, sem_b, sem_w, sem_out,
            *, seg, n_heads, dh):
    S, D = x_v.shape
    M = mem0_ref.shape[0]
    L = M + seg
    n_seg = S // seg
    n_pair = n_heads // 2
    PW = 2 * dh
    n_slab = D // LANES
    bdh = D // B_HEADS
    n_chunk = S // (2 * B_CHUNK)
    ppc = n_pair // n_chunk
    buf_a, buf_b = (q_a, k_a, v_a), (q_b, k_b, v_b)

    x_cuts = (0, 2 * B_CHUNK, 4 * B_CHUNK, S)
    cp_x0, cp_x1, cp_x2 = (
        pltpu.make_async_copy(x_hbm.at[lo:hi], x_v.at[lo:hi], sem_in.at[i])
        for i, (lo, hi) in enumerate(zip(x_cuts, x_cuts[1:])))
    cp_bwo = pltpu.make_async_copy(bwo_hbm, bwo_v, sem_in.at[3])

    def cp_bqkv(s):
        rows = pl.ds(s * LANES, LANES)
        return pltpu.make_async_copy(bqkv_hbm.at[rows], bqkv_v.at[rows],
                                     sem_b.at[s])

    def cp_w(c, j):
        rows = pl.ds(pl.multiple_of(c * ppc * PW, PW), ppc * PW)
        src = (wq_hbm, wk_hbm, wv_hbm, wo_hbm)[j]
        dst = wo_v.at[rows] if j == 3 else wraw.at[j, rows]
        return pltpu.make_async_copy(src.at[rows], dst, sem_w.at[c, j])

    for s in range(n_slab):
        cp_bqkv(s).start()
    cp_x0.start()
    for ref in buf_b:
        ref[...] = jnp.zeros(ref.shape, ref.dtype)

    for s in range(n_slab):
        cp_bqkv(s).wait()
        if s == n_slab - 1:
            cp_x1.start()
            cp_x2.start()
            for j in range(3):
                cp_w(0, j).start()
        slab[s, 0:3 * D, :] = bqkv_v[s * LANES:(s + 1) * LANES, :].astype(F32).T
        for part in range(3):
            for d in range(bdh):
                r0 = part * D + d * B_HEADS
                bqkv_p[r0:r0 + B_HEADS, s * LANES:(s + 1) * LANES] = slab[
                    s, pl.ds(part * D + d, B_HEADS, stride=bdh), :].astype(BF16)
    cp_x0.wait()

    bscale = bdh ** -0.5
    gate = gate_ref[...].astype(F32).reshape(1, D)

    def b_project(t0, dst, prev, is_first):
        for j in range(3):
            y = _dot_nt(x_v[pl.ds(t0, B_CHUNK), :], bqkv_p[j * D:(j + 1) * D, :])
            for s in range(n_slab):
                t = y[:, s * LANES:(s + 1) * LANES]
                if j == 0:
                    dst[j][s] = t
                    continue
                halo = prev[j][s, B_CHUNK:, :]
                if is_first is not None:
                    halo = jnp.where(
                        is_first, jnp.broadcast_to(t[0:1], halo.shape), halo)
                dst[j][s, 0:B_PAD, :] = halo
                dst[j][s, B_PAD:, :] = t
            yield

    def b_attend(t0, src):
        q_s, k_s, v_s = src
        for r in range(0, B_CHUNK, B_SUB):
            qs = [q_s[s, r:r + B_SUB, :] for s in range(n_slab)]
            logits = []
            for w in range(B_WIN):
                o = B_PAD + r - w * B_DIL
                acc = qs[0] * k_s[0, o:o + B_SUB, :]
                for s in range(1, n_slab):
                    acc = acc + qs[s] * k_s[s, o:o + B_SUB, :]
                acc = acc + pltpu.roll(acc, 64, 1)
                acc = acc + pltpu.roll(acc, 32, 1)
                if r < w * B_DIL:
                    pos = t0 + r + lax.broadcasted_iota(
                        jnp.int32, (B_SUB, LANES), 0)
                    acc = jnp.where(pos >= w * B_DIL, acc, NEG / bscale)
                logits.append(acc)
            mx = functools.reduce(jnp.maximum, logits)
            es = [jnp.exp2((l - mx) * (bscale * LOG2E)) for l in logits]
            inv = 1.0 / functools.reduce(jnp.add, es)
            cols = []
            for s in range(n_slab):
                acc = None
                for w in range(B_WIN):
                    o = B_PAD + r - w * B_DIL
                    t = es[w] * v_s[s, o:o + B_SUB, :]
                    acc = t if acc is None else acc + t
                cols.append((acc * inv).astype(BF16))
            ob_v[pl.ds(t0 + r, B_SUB), :] = jnp.concatenate(cols, axis=1)
            if (r // B_SUB) % 2:
                yield

    def prepare(c):
        for i in range(ppc):
            p = c * ppc + i
            tok = pl.ds(pl.multiple_of(p * (S // n_pair), S // n_pair),
                        S // n_pair)
            g = jax.nn.sigmoid(jnp.sum(x_v[tok, :].astype(F32) * gate,
                                       axis=-1, keepdims=True))
            g_v[tok, :] = jnp.broadcast_to(g, (S // n_pair, LANES))
            rows = pl.ds(pl.multiple_of(p * PW, PW), PW)
            qpre[p] = _dot_nt(xt_v[...], wraw[0, rows, :])
            yield
            for j in range(3):
                w_v[p, :, j * PW:(j + 1) * PW] = wraw[j, rows, :].T
            yield

    def b_body(c, carry):
        t0 = pl.multiple_of(c * 2 * B_CHUNK, B_CHUNK)
        t1 = pl.multiple_of(t0 + B_CHUNK, B_CHUNK)
        tp = pl.multiple_of(jnp.maximum(t0 - B_CHUNK, 0), B_CHUNK)
        _interleave(b_project(t0, buf_a, buf_b, c == 0), b_attend(tp, buf_b))
        _interleave(b_project(t1, buf_b, buf_a, None), b_attend(t0, buf_a))

        @pl.when(c == 1)
        def _():
            cp_x2.wait()
            for i in range(0, n_seg, 2):
                xt_v[i * PRE:(i + 2) * PRE, :] = jnp.concatenate(
                    [x_v[(i + u + 1) * seg - 2 * PRE:(i + u + 1) * seg, :]
                     .astype(F32)[PRE:] for u in range(2)], axis=0).astype(BF16)

        @pl.when(c == 0)
        def _():
            cp_x1.wait()

        @pl.when(c > 0)
        def _():
            for j in range(3):
                cp_w(c - 1, j).wait()

        @pl.when(c + 1 < n_chunk)
        def _():
            for j in range(3):
                cp_w(c + 1, j).start()

        cp_w(c, 3).start()

        @pl.when(c == n_chunk - 1)
        def _():
            cp_bwo.start()

        @pl.when(c > 0)
        def _():
            _interleave(prepare(c - 1))
        return carry

    lax.fori_loop(0, n_chunk, b_body, 0)

    def permute_bwo():
        for s in range(n_slab):
            slab[s, 0:D, :] = bwo_v[:, s * LANES:(s + 1) * LANES].astype(F32)
            for d in range(bdh):
                bwo_p[d * B_HEADS:(d + 1) * B_HEADS,
                      s * LANES:(s + 1) * LANES] = slab[
                    s, pl.ds(d, B_HEADS, stride=bdh), :].astype(BF16)
        yield

    cp_bwo.wait()
    for j in range(3):
        cp_w(n_chunk - 1, j).wait()
    _interleave(prepare(n_chunk - 1), permute_bwo(),
                b_attend(S - B_CHUNK, buf_b))
    for c in range(n_chunk):
        cp_w(c, 3).wait()

    scale = dh ** -0.5

    def step(s, mem):
        r0 = pl.multiple_of(s * seg, seg)
        h = jnp.concatenate([mem, x_v[pl.ds(r0, seg), :].astype(F32)], axis=0)

        row = lax.broadcasted_iota(jnp.int32, (L, 2 * L), 0)
        col = lax.broadcasted_iota(jnp.int32, (L, 2 * L), 1)
        first = col < L
        visible = (row < M) | (row >= jnp.where(first, col, col - L))
        lo = lax.broadcasted_iota(jnp.int32, (L, PW), 1) < dh

        def block_diag(t):
            return jnp.concatenate(
                [jnp.where(lo, t, 0.0), jnp.where(lo, 0.0, t)],
                axis=0).astype(BF16)

        def project(p):
            q = jnp.concatenate(
                [_dot(h[:L - PRE], w_v[p, :, :PW]),
                 qpre[p, pl.ds(pl.multiple_of(s * PRE, PRE), PRE), :]], axis=0)
            kv = _dot(h, w_v[p, :, PW:])
            return q, block_diag(kv[:, :PW]), block_diag(kv[:, PW:])

        def scores(q, kb):
            sc = jnp.where(visible, _dot_nt(q, kb) * scale, NEG)
            ma = jnp.max(jnp.where(first, sc, -jnp.inf), axis=-1, keepdims=True)
            mb = jnp.max(jnp.where(first, -jnp.inf, sc), axis=-1, keepdims=True)
            e = jnp.exp(sc - jnp.where(first, ma, mb))
            sa = jnp.sum(jnp.where(first, e, 0.0), axis=-1, keepdims=True)
            sb = jnp.sum(jnp.where(first, 0.0, e), axis=-1, keepdims=True)
            return e * jnp.where(first, 1.0 / sa, 1.0 / sb)

        proj, prob, outs = {}, {}, {}
        acc = None

        def out_proj(acc, pairs):
            for p in pairs:
                y = _dot(outs[p], wo_v[p * PW:(p + 1) * PW, :])
                acc = y if acc is None else acc + y
            return acc

        for t in range(n_pair + 2):
            if t < n_pair:
                proj[t] = project(t)
            if t == n_pair:
                acc = out_proj(acc, range(0, n_pair // 4))
            if 0 <= t - 1 < n_pair:
                prob[t - 1] = scores(proj[t - 1][0], proj[t - 1][1])
            if t == n_pair + 1:
                acc = out_proj(acc, range(n_pair // 4, n_pair - 4))
            if 0 <= t - 2 < n_pair:
                outs[t - 2] = _dot(prob[t - 2], proj[t - 2][2])
        acc = out_proj(acc, range(n_pair - 4, n_pair))

        b = _dot(ob_v[pl.ds(r0, seg), :], bwo_p[...])
        g = jnp.concatenate([g_v[pl.ds(r0, seg), :]] * n_slab, axis=1)
        out_v[pl.ds(r0, seg), :] = (
            g * acc[M:] + (1.0 - g) * b).astype(out_v.dtype)
        pltpu.make_async_copy(out_v.at[pl.ds(r0, seg)],
                              out_hbm.at[pl.ds(r0, seg)], sem_out.at[0]).start()
        return acc[:M]

    lax.fori_loop(0, n_seg, step, mem0_ref[...].astype(F32), unroll=UNROLL)
    pltpu.make_async_copy(out_v, out_v, sem_out.at[0]).wait()


@functools.partial(jax.jit, static_argnames=("A_seg_len",))
def pallas_gated_mix__memory_aug_recurrent_mem_tr__sliding_local_dilated__prompt_kernel(
    A_x: jax.Array,
    A_mem0: jax.Array,
    A_Wq: jax.Array,
    A_Wk: jax.Array,
    A_Wv: jax.Array,
    A_Wo: jax.Array,
    A_seg_len: int,
    B_x: jax.Array,
    B_wqkv: jax.Array,
    B_wo: jax.Array,
    gate_w: jax.Array,
):
    del B_x
    _, S, D = A_x.shape
    _, H, Dh = A_Wq.shape
    M = A_mem0.shape[1]
    seg = int(A_seg_len)
    n_pair = H // 2
    n_slab = D // LANES
    n_chunk = S // (2 * B_CHUNK)

    def by_head(w):
        return jnp.transpose(w, (1, 2, 0)).reshape(H * Dh, D)

    qkv_buf = [pltpu.VMEM((n_slab, B_CHUNK, LANES), F32),
               pltpu.VMEM((n_slab, B_CHUNK + B_PAD, LANES), F32),
               pltpu.VMEM((n_slab, B_CHUNK + B_PAD, LANES), F32)]
    hbm = pl.BlockSpec(memory_space=pl.ANY)
    vmem = pl.BlockSpec(memory_space=pltpu.VMEM)
    out = pl.pallas_call(
        functools.partial(_kernel, seg=seg, n_heads=H, dh=Dh),
        out_shape=jax.ShapeDtypeStruct((S, D), A_x.dtype),
        in_specs=[hbm, vmem, hbm, hbm, hbm, hbm, hbm, hbm, vmem],
        out_specs=hbm,
        scratch_shapes=[
            pltpu.VMEM((S, D), BF16),
            pltpu.VMEM((S // seg * PRE, D), BF16),
            pltpu.VMEM((3, H * Dh, D), BF16),
            pltpu.VMEM((n_pair, D, 6 * Dh), BF16),
            pltpu.VMEM((H * Dh, D), BF16),
            pltpu.VMEM((D, 3 * D), BF16),
            pltpu.VMEM((D, D), BF16),
            pltpu.VMEM((n_slab, 3 * D + B_HEADS, LANES), F32),
            pltpu.VMEM((3 * D, D), BF16),
            pltpu.VMEM((D, D), BF16),
            *qkv_buf, *qkv_buf,
            pltpu.VMEM((S, LANES), F32),
            pltpu.VMEM((S, D), BF16),
            pltpu.VMEM((n_pair, S // seg * PRE, 2 * Dh), F32),
            pltpu.VMEM((S, D), A_x.dtype),
            pltpu.SemaphoreType.DMA((4,)),
            pltpu.SemaphoreType.DMA((n_slab,)),
            pltpu.SemaphoreType.DMA((n_chunk, 4)),
            pltpu.SemaphoreType.DMA((1,)),
        ],
        compiler_params=pltpu.CompilerParams(
            vmem_limit_bytes=110 * 1024 * 1024),
    )(A_x.reshape(S, D), A_mem0.reshape(M, D), by_head(A_Wq), by_head(A_Wk),
      by_head(A_Wv), A_Wo.reshape(H * Dh, D), B_wqkv, B_wo,
      gate_w)
    return out.reshape(1, S, D)
```

```python
import functools

import jax
import jax.numpy as jnp
from jax import lax
import jax.experimental.pallas as pl
import jax.experimental.pallas.tpu as pltpu

F32 = jnp.float32
BF16 = jnp.bfloat16
LANES = 128
NEG = -1000000000.0
LOG2E = 1.4426950408889634

B_HEADS = 32
B_WIN = 8
B_DIL = 2
B_PAD = 16
B_CHUNK = 128
PRE = 8
UNROLL = 4
LAG = 2
B_SUB = 32


def _dot(a, b):
    return lax.dot_general(a, b, (((1,), (0,)), ((), ())),
                           preferred_element_type=F32)


def _dot_nt(a, b):
    return lax.dot_general(a, b, (((1,), (1,)), ((), ())),
                           preferred_element_type=F32)


def _interleave(*stages):
    stages = list(stages)
    while stages:
        for g in list(stages):
            if next(g, _DONE) is _DONE:
                stages.remove(g)


_DONE = object()


def _kernel(x_hbm, mem0_ref, wq_hbm, wk_hbm, wv_hbm, wo_hbm, bqkv_hbm, bwo_hbm,
            gate_ref, out_hbm,
            x_v, xt_v, wraw, w_v, wo_v, bqkv_v, bwo_v, slab, bqkv_p, bwo_p,
            q_a, k_a, v_a, q_b, k_b, v_b, g_v, ob_v, qpre, out_v,
            sem_in, sem_b, sem_w, sem_out,
            *, seg, n_heads, dh):
    S, D = x_v.shape
    M = mem0_ref.shape[0]
    L = M + seg
    n_seg = S // seg
    n_pair = n_heads // 2
    PW = 2 * dh
    n_slab = D // LANES
    bdh = D // B_HEADS
    n_chunk = S // (2 * B_CHUNK)
    ppc = n_pair // n_chunk
    buf_a, buf_b = (q_a, k_a, v_a), (q_b, k_b, v_b)

    x_cuts = (0, 2 * B_CHUNK, 2 * (LAG + 1) * B_CHUNK, S)
    cp_x0, cp_x1, cp_x2 = (
        pltpu.make_async_copy(x_hbm.at[lo:hi], x_v.at[lo:hi], sem_in.at[i])
        for i, (lo, hi) in enumerate(zip(x_cuts, x_cuts[1:])))
    cp_bwo = pltpu.make_async_copy(bwo_hbm, bwo_v, sem_in.at[3])

    def cp_bqkv(s):
        rows = pl.ds(s * LANES, LANES)
        return pltpu.make_async_copy(bqkv_hbm.at[rows], bqkv_v.at[rows],
                                     sem_b.at[s])

    def cp_w(c, j):
        rows = pl.ds(pl.multiple_of(c * ppc * PW, PW), ppc * PW)
        src = (wq_hbm, wk_hbm, wv_hbm, wo_hbm)[j]
        dst = wo_v.at[rows] if j == 3 else wraw.at[j, rows]
        return pltpu.make_async_copy(src.at[rows], dst, sem_w.at[c, j])

    for s in range(n_slab):
        cp_bqkv(s).start()
    cp_x0.start()
    for ref in buf_b:
        ref[...] = jnp.zeros(ref.shape, ref.dtype)

    for s in range(n_slab):
        cp_bqkv(s).wait()
        if s == n_slab - 1:
            cp_x1.start()
            cp_x2.start()
            for j in range(3):
                cp_w(0, j).start()
        slab[s, 0:3 * D, :] = bqkv_v[s * LANES:(s + 1) * LANES, :].astype(F32).T
        for part in range(3):
            for d in range(bdh):
                r0 = part * D + d * B_HEADS
                bqkv_p[r0:r0 + B_HEADS, s * LANES:(s + 1) * LANES] = slab[
                    s, pl.ds(part * D + d, B_HEADS, stride=bdh), :].astype(BF16)
    cp_x0.wait()

    bscale = bdh ** -0.5
    gate = gate_ref[...].astype(F32).reshape(1, D)

    def b_project(t0, dst, prev, is_first):
        for j in range(3):
            y = _dot_nt(x_v[pl.ds(t0, B_CHUNK), :], bqkv_p[j * D:(j + 1) * D, :])
            for s in range(n_slab):
                t = y[:, s * LANES:(s + 1) * LANES]
                if j == 0:
                    dst[j][s] = t
                    continue
                halo = prev[j][s, B_CHUNK:, :]
                if is_first is not None:
                    halo = jnp.where(
                        is_first, jnp.broadcast_to(t[0:1], halo.shape), halo)
                dst[j][s, 0:B_PAD, :] = halo
                dst[j][s, B_PAD:, :] = t
            yield

    def b_attend(t0, src):
        q_s, k_s, v_s = src
        for r in range(0, B_CHUNK, B_SUB):
            qs = [q_s[s, r:r + B_SUB, :] for s in range(n_slab)]
            logits = []
            for w in range(B_WIN):
                o = B_PAD + r - w * B_DIL
                acc = qs[0] * k_s[0, o:o + B_SUB, :]
                for s in range(1, n_slab):
                    acc = acc + qs[s] * k_s[s, o:o + B_SUB, :]
                acc = acc + pltpu.roll(acc, 64, 1)
                acc = acc + pltpu.roll(acc, 32, 1)
                if r < w * B_DIL:
                    pos = t0 + r + lax.broadcasted_iota(
                        jnp.int32, (B_SUB, LANES), 0)
                    acc = jnp.where(pos >= w * B_DIL, acc, NEG / bscale)
                logits.append(acc)
            mx = functools.reduce(jnp.maximum, logits)
            es = [jnp.exp2((l - mx) * (bscale * LOG2E)) for l in logits]
            inv = 1.0 / functools.reduce(jnp.add, es)
            cols = []
            for s in range(n_slab):
                acc = None
                for w in range(B_WIN):
                    o = B_PAD + r - w * B_DIL
                    t = es[w] * v_s[s, o:o + B_SUB, :]
                    acc = t if acc is None else acc + t
                cols.append((acc * inv).astype(BF16))
            ob_v[pl.ds(t0 + r, B_SUB), :] = jnp.concatenate(cols, axis=1)
            if (r // B_SUB) % 2:
                yield

    def prepare(c):
        for i in range(ppc):
            p = c * ppc + i
            tok = pl.ds(pl.multiple_of(p * (S // n_pair), S // n_pair),
                        S // n_pair)
            g = jax.nn.sigmoid(jnp.sum(x_v[tok, :].astype(F32) * gate,
                                       axis=-1, keepdims=True))
            g_v[tok, :] = jnp.broadcast_to(g, (S // n_pair, LANES))
            rows = pl.ds(pl.multiple_of(p * PW, PW), PW)
            qpre[p] = _dot_nt(xt_v[...], wraw[0, rows, :])
            yield
            for j in range(3):
                w_v[p, :, j * PW:(j + 1) * PW] = wraw[j, rows, :].T
            yield

    def b_body(c, carry):
        t0 = pl.multiple_of(c * 2 * B_CHUNK, B_CHUNK)
        t1 = pl.multiple_of(t0 + B_CHUNK, B_CHUNK)
        tp = pl.multiple_of(jnp.maximum(t0 - B_CHUNK, 0), B_CHUNK)
        _interleave(b_project(t0, buf_a, buf_b, c == 0), b_attend(tp, buf_b))
        _interleave(b_project(t1, buf_b, buf_a, None), b_attend(t0, buf_a))

        @pl.when(c == LAG)
        def _():
            cp_x2.wait()
            for i in range(0, n_seg, 2):
                xt_v[i * PRE:(i + 2) * PRE, :] = jnp.concatenate(
                    [x_v[(i + u + 1) * seg - 2 * PRE:(i + u + 1) * seg, :]
                     .astype(F32)[PRE:] for u in range(2)], axis=0).astype(BF16)

        @pl.when(c == 0)
        def _():
            cp_x1.wait()

        @pl.when(c >= LAG)
        def _():
            for j in range(3):
                cp_w(c - LAG, j).wait()

        @pl.when(c + 1 < n_chunk)
        def _():
            for j in range(3):
                cp_w(c + 1, j).start()

        cp_w(c, 3).start()

        @pl.when(c == n_chunk - 1)
        def _():
            cp_bwo.start()

        @pl.when(c >= LAG)
        def _():
            _interleave(prepare(c - LAG))
        return carry

    lax.fori_loop(0, n_chunk, b_body, 0)

    def permute_bwo():
        for s in range(n_slab):
            slab[s, 0:D, :] = bwo_v[:, s * LANES:(s + 1) * LANES].astype(F32)
            for d in range(bdh):
                bwo_p[d * B_HEADS:(d + 1) * B_HEADS,
                      s * LANES:(s + 1) * LANES] = slab[
                    s, pl.ds(d, B_HEADS, stride=bdh), :].astype(BF16)
        yield

    cp_bwo.wait()
    for c in range(n_chunk - LAG, n_chunk):
        for j in range(3):
            cp_w(c, j).wait()
    _interleave(prepare(n_chunk - LAG), permute_bwo(),
                b_attend(S - B_CHUNK, buf_b))
    for c in range(n_chunk - LAG + 1, n_chunk):
        _interleave(prepare(c))
    for c in range(n_chunk):
        cp_w(c, 3).wait()

    scale = dh ** -0.5

    def step(s, mem):
        r0 = pl.multiple_of(s * seg, seg)
        h = jnp.concatenate([mem, x_v[pl.ds(r0, seg), :].astype(F32)], axis=0)

        row = lax.broadcasted_iota(jnp.int32, (L, 2 * L), 0)
        col = lax.broadcasted_iota(jnp.int32, (L, 2 * L), 1)
        first = col < L
        visible = (row < M) | (row >= jnp.where(first, col, col - L))
        lo = lax.broadcasted_iota(jnp.int32, (L, PW), 1) < dh

        def block_diag(t):
            return jnp.concatenate(
                [jnp.where(lo, t, 0.0), jnp.where(lo, 0.0, t)],
                axis=0).astype(BF16)

        def project(p):
            q = jnp.concatenate(
                [_dot(h[:L - PRE], w_v[p, :, :PW]),
                 qpre[p, pl.ds(pl.multiple_of(s * PRE, PRE), PRE), :]], axis=0)
            kv = _dot(h, w_v[p, :, PW:])
            return q, block_diag(kv[:, :PW]), block_diag(kv[:, PW:])

        def scores(q, kb):
            sc = jnp.where(visible, _dot_nt(q, kb) * scale, NEG)
            ma = jnp.max(jnp.where(first, sc, -jnp.inf), axis=-1, keepdims=True)
            mb = jnp.max(jnp.where(first, -jnp.inf, sc), axis=-1, keepdims=True)
            e = jnp.exp(sc - jnp.where(first, ma, mb))
            sa = jnp.sum(jnp.where(first, e, 0.0), axis=-1, keepdims=True)
            sb = jnp.sum(jnp.where(first, 0.0, e), axis=-1, keepdims=True)
            return e * jnp.where(first, 1.0 / sa, 1.0 / sb)

        proj, prob, outs = {}, {}, {}
        acc = None

        def out_proj(acc, pairs):
            for p in pairs:
                y = _dot(outs[p], wo_v[p * PW:(p + 1) * PW, :])
                acc = y if acc is None else acc + y
            return acc

        for t in range(n_pair + 2):
            if t < n_pair:
                proj[t] = project(t)
            if t == n_pair:
                acc = out_proj(acc, range(0, n_pair // 4))
            if 0 <= t - 1 < n_pair:
                prob[t - 1] = scores(proj[t - 1][0], proj[t - 1][1])
            if t == n_pair + 1:
                acc = out_proj(acc, range(n_pair // 4, n_pair - 4))
            if 0 <= t - 2 < n_pair:
                outs[t - 2] = _dot(prob[t - 2], proj[t - 2][2])
        acc = out_proj(acc, range(n_pair - 4, n_pair))

        b = _dot(ob_v[pl.ds(r0, seg), :], bwo_p[...])
        g = jnp.concatenate([g_v[pl.ds(r0, seg), :]] * n_slab, axis=1)
        out_v[pl.ds(r0, seg), :] = (
            g * acc[M:] + (1.0 - g) * b).astype(out_v.dtype)
        pltpu.make_async_copy(out_v.at[pl.ds(r0, seg)],
                              out_hbm.at[pl.ds(r0, seg)], sem_out.at[0]).start()
        return acc[:M]

    lax.fori_loop(0, n_seg, step, mem0_ref[...].astype(F32), unroll=UNROLL)
    pltpu.make_async_copy(out_v, out_v, sem_out.at[0]).wait()


@functools.partial(jax.jit, static_argnames=("A_seg_len",))
def pallas_gated_mix__memory_aug_recurrent_mem_tr__sliding_local_dilated__prompt_kernel(
    A_x: jax.Array,
    A_mem0: jax.Array,
    A_Wq: jax.Array,
    A_Wk: jax.Array,
    A_Wv: jax.Array,
    A_Wo: jax.Array,
    A_seg_len: int,
    B_x: jax.Array,
    B_wqkv: jax.Array,
    B_wo: jax.Array,
    gate_w: jax.Array,
):
    del B_x
    _, S, D = A_x.shape
    _, H, Dh = A_Wq.shape
    M = A_mem0.shape[1]
    seg = int(A_seg_len)
    n_pair = H // 2
    n_slab = D // LANES
    n_chunk = S // (2 * B_CHUNK)

    def by_head(w):
        return jnp.transpose(w, (1, 2, 0)).reshape(H * Dh, D)

    qkv_buf = [pltpu.VMEM((n_slab, B_CHUNK, LANES), F32),
               pltpu.VMEM((n_slab, B_CHUNK + B_PAD, LANES), F32),
               pltpu.VMEM((n_slab, B_CHUNK + B_PAD, LANES), F32)]
    hbm = pl.BlockSpec(memory_space=pl.ANY)
    vmem = pl.BlockSpec(memory_space=pltpu.VMEM)
    out = pl.pallas_call(
        functools.partial(_kernel, seg=seg, n_heads=H, dh=Dh),
        out_shape=jax.ShapeDtypeStruct((S, D), A_x.dtype),
        in_specs=[hbm, vmem, hbm, hbm, hbm, hbm, hbm, hbm, vmem],
        out_specs=hbm,
        scratch_shapes=[
            pltpu.VMEM((S, D), BF16),
            pltpu.VMEM((S // seg * PRE, D), BF16),
            pltpu.VMEM((3, H * Dh, D), BF16),
            pltpu.VMEM((n_pair, D, 6 * Dh), BF16),
            pltpu.VMEM((H * Dh, D), BF16),
            pltpu.VMEM((D, 3 * D), BF16),
            pltpu.VMEM((D, D), BF16),
            pltpu.VMEM((n_slab, 3 * D + B_HEADS, LANES), F32),
            pltpu.VMEM((3 * D, D), BF16),
            pltpu.VMEM((D, D), BF16),
            *qkv_buf, *qkv_buf,
            pltpu.VMEM((S, LANES), F32),
            pltpu.VMEM((S, D), BF16),
            pltpu.VMEM((n_pair, S // seg * PRE, 2 * Dh), F32),
            pltpu.VMEM((S, D), A_x.dtype),
            pltpu.SemaphoreType.DMA((4,)),
            pltpu.SemaphoreType.DMA((n_slab,)),
            pltpu.SemaphoreType.DMA((n_chunk, 4)),
            pltpu.SemaphoreType.DMA((1,)),
        ],
        compiler_params=pltpu.CompilerParams(
            vmem_limit_bytes=110 * 1024 * 1024),
    )(A_x.reshape(S, D), A_mem0.reshape(M, D), by_head(A_Wq), by_head(A_Wk),
      by_head(A_Wv), A_Wo.reshape(H * Dh, D), B_wqkv, B_wo,
      gate_w)
    return out.reshape(1, S, D)
```

```python
import functools

import jax
import jax.numpy as jnp
from jax import lax
import jax.experimental.pallas as pl
import jax.experimental.pallas.tpu as pltpu

F32 = jnp.float32
BF16 = jnp.bfloat16
LANES = 128
NEG = -1000000000.0
LOG2E = 1.4426950408889634

B_HEADS = 32
B_WIN = 8
B_DIL = 2
B_PAD = 16
B_CHUNK = 128
PRE = 8
UNROLL = 4
N_EARLY = 3
B_SUB = 32


def _dot(a, b):
    return lax.dot_general(a, b, (((1,), (0,)), ((), ())),
                           preferred_element_type=F32)


def _dot_nt(a, b):
    return lax.dot_general(a, b, (((1,), (1,)), ((), ())),
                           preferred_element_type=F32)


def _interleave(*stages):
    stages = list(stages)
    while stages:
        for g in list(stages):
            if next(g, _DONE) is _DONE:
                stages.remove(g)


_DONE = object()


def _kernel(x_hbm, mem0_ref, wq_hbm, wk_hbm, wv_hbm, wo_hbm, bqkv_hbm, bwo_hbm,
            gate_ref, out_hbm,
            x_v, xt_v, wraw, w_v, wo_v, bqkv_v, bwo_v, slab, bqkv_p, bwo_p,
            q_a, k_a, v_a, q_b, k_b, v_b, g_v, ob_v, qpre, out_v,
            sem_in, sem_b, sem_w, sem_out,
            *, seg, n_heads, dh):
    S, D = x_v.shape
    M = mem0_ref.shape[0]
    L = M + seg
    n_seg = S // seg
    n_pair = n_heads // 2
    PW = 2 * dh
    n_slab = D // LANES
    bdh = D // B_HEADS
    n_chunk = S // (2 * B_CHUNK)
    n_late = n_chunk - N_EARLY
    ppc = n_pair // n_late
    buf_a, buf_b = (q_a, k_a, v_a), (q_b, k_b, v_b)

    x_cuts = (0, 2 * B_CHUNK, 2 * N_EARLY * B_CHUNK, S)
    cp_x0, cp_x1, cp_x2 = (
        pltpu.make_async_copy(x_hbm.at[lo:hi], x_v.at[lo:hi], sem_in.at[i])
        for i, (lo, hi) in enumerate(zip(x_cuts, x_cuts[1:])))
    cp_bwo = pltpu.make_async_copy(bwo_hbm, bwo_v, sem_in.at[3])
    cp_wo = pltpu.make_async_copy(wo_hbm, wo_v, sem_in.at[4])

    def cp_bqkv(s):
        rows = pl.ds(pl.multiple_of(s * LANES, LANES), LANES)
        return pltpu.make_async_copy(bqkv_hbm.at[rows], bqkv_v.at[rows],
                                     sem_b.at[s])

    def cp_w(i):
        last = isinstance(i, int) and i == n_late
        n = (n_pair - n_late * ppc if last else ppc) * PW
        rows = pl.ds(pl.multiple_of(i * ppc * PW, PW), n)
        return [pltpu.make_async_copy(src.at[rows], wraw.at[j, rows],
                                      sem_w.at[i, j])
                for j, src in enumerate((wq_hbm, wk_hbm, wv_hbm))]

    for s in range(n_slab):
        cp_bqkv(s).start()
    cp_x0.start()
    for ref in buf_b:
        ref[...] = jnp.zeros(ref.shape, ref.dtype)

    def permute_bqkv(s, carry):
        cp_bqkv(s).wait()

        @pl.when(s == n_slab - 1)
        def _():
            cp_x1.start()
            cp_x2.start()
            for cp in cp_w(0):
                cp.start()

        rows = pl.ds(pl.multiple_of(s * LANES, LANES), LANES)
        slab[0, 0:3 * D, :] = bqkv_v[rows, :].astype(F32).T
        for part in range(3):
            for d in range(bdh):
                r0 = part * D + d * B_HEADS
                bqkv_p[s, r0:r0 + B_HEADS, :] = slab[
                    0, pl.ds(part * D + d, B_HEADS, stride=bdh), :].astype(BF16)
        return carry

    lax.fori_loop(0, n_slab, permute_bqkv, 0)
    cp_x0.wait()

    bscale = bdh ** -0.5
    gate = gate_ref[...].astype(F32).reshape(1, D)

    def b_project(t0, dst, prev, is_first):
        for j in range(3):
            w = jnp.concatenate(
                [bqkv_p[s, j * D:(j + 1) * D, :] for s in range(n_slab)], axis=1)
            y = _dot_nt(x_v[pl.ds(t0, B_CHUNK), :], w)
            for s in range(n_slab):
                t = y[:, s * LANES:(s + 1) * LANES]
                if j == 0:
                    dst[j][s] = t
                    continue
                halo = prev[j][s, B_CHUNK:, :]
                if is_first is not None:
                    halo = jnp.where(
                        is_first, jnp.broadcast_to(t[0:1], halo.shape), halo)
                dst[j][s, 0:B_PAD, :] = halo
                dst[j][s, B_PAD:, :] = t
            yield

    def b_attend(t0, src):
        q_s, k_s, v_s = src
        for r in range(0, B_CHUNK, B_SUB):
            qs = [q_s[s, r:r + B_SUB, :] for s in range(n_slab)]
            logits = []
            for w in range(B_WIN):
                o = B_PAD + r - w * B_DIL
                acc = qs[0] * k_s[0, o:o + B_SUB, :]
                for s in range(1, n_slab):
                    acc = acc + qs[s] * k_s[s, o:o + B_SUB, :]
                acc = acc + pltpu.roll(acc, 64, 1)
                acc = acc + pltpu.roll(acc, 32, 1)
                if r < w * B_DIL:
                    pos = t0 + r + lax.broadcasted_iota(
                        jnp.int32, (B_SUB, LANES), 0)
                    acc = jnp.where(pos >= w * B_DIL, acc, NEG / bscale)
                logits.append(acc)
            mx = functools.reduce(jnp.maximum, logits)
            es = [jnp.exp2((l - mx) * (bscale * LOG2E)) for l in logits]
            inv = 1.0 / functools.reduce(jnp.add, es)
            cols = []
            for s in range(n_slab):
                acc = None
                for w in range(B_WIN):
                    o = B_PAD + r - w * B_DIL
                    t = es[w] * v_s[s, o:o + B_SUB, :]
                    acc = t if acc is None else acc + t
                cols.append((acc * inv).astype(BF16))
            ob_v[pl.ds(t0 + r, B_SUB), :] = jnp.concatenate(cols, axis=1)
            if (r // B_SUB) % 2:
                yield

    def prepare(pairs):
        for p in pairs:
            tok = pl.ds(pl.multiple_of(p * (S // n_pair), S // n_pair),
                        S // n_pair)
            g = jax.nn.sigmoid(jnp.sum(x_v[tok, :].astype(F32) * gate,
                                       axis=-1, keepdims=True))
            g_v[tok, :] = jnp.broadcast_to(g, (S // n_pair, LANES))
            rows = pl.ds(pl.multiple_of(p * PW, PW), PW)
            qpre[p] = _dot_nt(xt_v[...], wraw[0, rows, :])
            yield
            for j in range(3):
                w_v[p, :, j * PW:(j + 1) * PW] = wraw[j, rows, :].T
            yield

    def b_chunks(c, is_first):
        t0 = pl.multiple_of(c * 2 * B_CHUNK, B_CHUNK)
        t1 = pl.multiple_of(t0 + B_CHUNK, B_CHUNK)
        tp = pl.multiple_of(jnp.maximum(t0 - B_CHUNK, 0), B_CHUNK)
        _interleave(b_project(t0, buf_a, buf_b, is_first), b_attend(tp, buf_b))
        _interleave(b_project(t1, buf_b, buf_a, None), b_attend(t0, buf_a))

    def early_body(c, carry):
        b_chunks(c, c == 0)

        @pl.when(c == 0)
        def _():
            cp_x1.wait()

        @pl.when(c == N_EARLY - 2)
        def _():
            for cp in cp_w(1):
                cp.start()

        return carry

    lax.fori_loop(0, N_EARLY, early_body, 0)
    cp_x2.wait()
    def gather_tail(i, carry):
        parts = []
        for u in range(2):
            r = pl.multiple_of((2 * i + u + 1) * seg - 2 * PRE, 2 * PRE)
            parts.append(x_v[pl.ds(r, 2 * PRE), :].astype(F32)[PRE:])
        xt_v[pl.ds(pl.multiple_of(i * 2 * PRE, 2 * PRE), 2 * PRE), :] = (
            jnp.concatenate(parts, axis=0).astype(BF16))
        return carry

    lax.fori_loop(0, n_seg // 2, gather_tail, 0, unroll=8)

    def late_body(i, carry):
        for cp in cp_w(i):
            cp.wait()

        @pl.when(i + 2 < n_late)
        def _():
            for cp in cp_w(i + 2):
                cp.start()

        @pl.when(i + 2 == n_late)
        def _():
            cp_bwo.start()
            for cp in cp_w(n_late):
                cp.start()
            cp_wo.start()

        _interleave(prepare([i * ppc + u for u in range(ppc)]))
        b_chunks(i + N_EARLY, None)
        return carry

    lax.fori_loop(0, n_late, late_body, 0)

    def permute_bwo():
        for s in range(n_slab):
            slab[s, 0:D, :] = bwo_v[:, s * LANES:(s + 1) * LANES].astype(F32)
            for d in range(bdh):
                bwo_p[d * B_HEADS:(d + 1) * B_HEADS,
                      s * LANES:(s + 1) * LANES] = slab[
                    s, pl.ds(d, B_HEADS, stride=bdh), :].astype(BF16)
        yield

    cp_bwo.wait()
    for cp in cp_w(n_late):
        cp.wait()
    _interleave(prepare(range(n_late * ppc, n_pair)), permute_bwo(),
                b_attend(S - B_CHUNK, buf_b))
    cp_wo.wait()

    scale = dh ** -0.5

    def step(s, mem):
        r0 = pl.multiple_of(s * seg, seg)
        h = jnp.concatenate([mem, x_v[pl.ds(r0, seg), :].astype(F32)], axis=0)

        row = lax.broadcasted_iota(jnp.int32, (L, 2 * L), 0)
        col = lax.broadcasted_iota(jnp.int32, (L, 2 * L), 1)
        first = col < L
        visible = (row < M) | (row >= jnp.where(first, col, col - L))
        lo = lax.broadcasted_iota(jnp.int32, (L, PW), 1) < dh

        def block_diag(t):
            return jnp.concatenate(
                [jnp.where(lo, t, 0.0), jnp.where(lo, 0.0, t)],
                axis=0).astype(BF16)

        def project(p):
            q = jnp.concatenate(
                [_dot(h[:L - PRE], w_v[p, :, :PW]),
                 qpre[p, pl.ds(pl.multiple_of(s * PRE, PRE), PRE), :]], axis=0)
            kv = _dot(h, w_v[p, :, PW:])
            return q, block_diag(kv[:, :PW]), block_diag(kv[:, PW:])

        def scores(q, kb):
            sc = jnp.where(visible, _dot_nt(q, kb) * scale, NEG)
            ma = jnp.max(jnp.where(first, sc, -jnp.inf), axis=-1, keepdims=True)
            mb = jnp.max(jnp.where(first, -jnp.inf, sc), axis=-1, keepdims=True)
            e = jnp.exp(sc - jnp.where(first, ma, mb))
            sa = jnp.sum(jnp.where(first, e, 0.0), axis=-1, keepdims=True)
            sb = jnp.sum(jnp.where(first, 0.0, e), axis=-1, keepdims=True)
            return e * jnp.where(first, 1.0 / sa, 1.0 / sb)

        proj, prob, outs = {}, {}, {}
        acc = None

        def out_proj(acc, pairs):
            for p in pairs:
                y = _dot(outs[p], wo_v[p * PW:(p + 1) * PW, :])
                acc = y if acc is None else acc + y
            return acc

        for t in range(n_pair + 2):
            if t < n_pair:
                proj[t] = project(t)
            if t == n_pair:
                acc = out_proj(acc, range(0, n_pair // 4))
            if 0 <= t - 1 < n_pair:
                prob[t - 1] = scores(proj[t - 1][0], proj[t - 1][1])
            if t == n_pair + 1:
                acc = out_proj(acc, range(n_pair // 4, n_pair - 4))
            if 0 <= t - 2 < n_pair:
                outs[t - 2] = _dot(prob[t - 2], proj[t - 2][2])
        acc = out_proj(acc, range(n_pair - 4, n_pair))

        b = _dot(ob_v[pl.ds(r0, seg), :], bwo_p[...])
        g = jnp.concatenate([g_v[pl.ds(r0, seg), :]] * n_slab, axis=1)
        out_v[pl.ds(r0, seg), :] = (
            g * acc[M:] + (1.0 - g) * b).astype(out_v.dtype)
        pltpu.make_async_copy(out_v.at[pl.ds(r0, seg)],
                              out_hbm.at[pl.ds(r0, seg)], sem_out.at[0]).start()
        return acc[:M]

    lax.fori_loop(0, n_seg, step, mem0_ref[...].astype(F32), unroll=UNROLL)
    pltpu.make_async_copy(out_v, out_v, sem_out.at[0]).wait()


@functools.partial(jax.jit, static_argnames=("A_seg_len",))
def pallas_gated_mix__memory_aug_recurrent_mem_tr__sliding_local_dilated__prompt_kernel(
    A_x: jax.Array,
    A_mem0: jax.Array,
    A_Wq: jax.Array,
    A_Wk: jax.Array,
    A_Wv: jax.Array,
    A_Wo: jax.Array,
    A_seg_len: int,
    B_x: jax.Array,
    B_wqkv: jax.Array,
    B_wo: jax.Array,
    gate_w: jax.Array,
):
    del B_x
    _, S, D = A_x.shape
    _, H, Dh = A_Wq.shape
    M = A_mem0.shape[1]
    seg = int(A_seg_len)
    n_pair = H // 2
    n_slab = D // LANES
    n_chunk = S // (2 * B_CHUNK)

    def by_head(w):
        return jnp.transpose(w, (1, 2, 0)).reshape(H * Dh, D)

    qkv_buf = [pltpu.VMEM((n_slab, B_CHUNK, LANES), F32),
               pltpu.VMEM((n_slab, B_CHUNK + B_PAD, LANES), F32),
               pltpu.VMEM((n_slab, B_CHUNK + B_PAD, LANES), F32)]
    hbm = pl.BlockSpec(memory_space=pl.ANY)
    vmem = pl.BlockSpec(memory_space=pltpu.VMEM)
    out = pl.pallas_call(
        functools.partial(_kernel, seg=seg, n_heads=H, dh=Dh),
        out_shape=jax.ShapeDtypeStruct((S, D), A_x.dtype),
        in_specs=[hbm, vmem, hbm, hbm, hbm, hbm, hbm, hbm, vmem],
        out_specs=hbm,
        scratch_shapes=[
            pltpu.VMEM((S, D), BF16),
            pltpu.VMEM((S // seg * PRE, D), BF16),
            pltpu.VMEM((3, H * Dh, D), BF16),
            pltpu.VMEM((n_pair, D, 6 * Dh), BF16),
            pltpu.VMEM((H * Dh, D), BF16),
            pltpu.VMEM((D, 3 * D), BF16),
            pltpu.VMEM((D, D), BF16),
            pltpu.VMEM((n_slab, 3 * D + B_HEADS, LANES), F32),
            pltpu.VMEM((n_slab, 3 * D, LANES), BF16),
            pltpu.VMEM((D, D), BF16),
            *qkv_buf, *qkv_buf,
            pltpu.VMEM((S, LANES), F32),
            pltpu.VMEM((S, D), BF16),
            pltpu.VMEM((n_pair, S // seg * PRE, 2 * Dh), F32),
            pltpu.VMEM((S, D), A_x.dtype),
            pltpu.SemaphoreType.DMA((5,)),
            pltpu.SemaphoreType.DMA((n_slab,)),
            pltpu.SemaphoreType.DMA((n_chunk - N_EARLY + 1, 3)),
            pltpu.SemaphoreType.DMA((1,)),
        ],
        compiler_params=pltpu.CompilerParams(
            vmem_limit_bytes=110 * 1024 * 1024),
    )(A_x.reshape(S, D), A_mem0.reshape(M, D), by_head(A_Wq), by_head(A_Wk),
      by_head(A_Wv), A_Wo.reshape(H * Dh, D), B_wqkv, B_wo,
      gate_w)
    return out.reshape(1, S, D)
```

```python
import functools

import jax
import jax.numpy as jnp
from jax import lax
import jax.experimental.pallas as pl
import jax.experimental.pallas.tpu as pltpu

F32 = jnp.float32
BF16 = jnp.bfloat16
LANES = 128
NEG = -1000000000.0
LOG2E = 1.4426950408889634

B_HEADS = 32
B_WIN = 8
B_DIL = 2
B_PAD = 16
B_CHUNK = 128
B_SUB = 32
N_EARLY = 2
PRE = 8
UNROLL = 4


def _dot(a, b):
    return lax.dot_general(a, b, (((1,), (0,)), ((), ())),
                           preferred_element_type=F32)


def _dot_nt(a, b):
    return lax.dot_general(a, b, (((1,), (1,)), ((), ())),
                           preferred_element_type=F32)


def _interleave(*stages):
    stages = list(stages)
    while stages:
        for g in list(stages):
            if next(g, _DONE) is _DONE:
                stages.remove(g)


_DONE = object()


def _kernel(x_hbm, mem0_ref, wq_hbm, wk_hbm, wv_hbm, wo_hbm, bqkv_hbm, bwo_hbm,
            gate_ref, out_hbm,
            x_v, xt_v, wraw, w_v, wo_v, bqkv_v, bwo_v, slab, bqkv_p, bwo_p,
            q_a, k_a, v_a, q_b, k_b, v_b, g_v, ob_v, qpre, out_v,
            sem_in, sem_b, sem_w, sem_out,
            *, seg, n_heads, dh):
    S, D = x_v.shape
    M = mem0_ref.shape[0]
    L = M + seg
    n_seg = S // seg
    n_pair = n_heads // 2
    PW = 2 * dh
    n_slab = D // LANES
    bdh = D // B_HEADS
    n_chunk = S // (2 * B_CHUNK)
    n_late = n_chunk - N_EARLY
    assert n_late >= n_slab
    ppc = n_pair // n_late
    buf_a, buf_b = (q_a, k_a, v_a), (q_b, k_b, v_b)

    x_cuts = (0, 2 * B_CHUNK, 2 * N_EARLY * B_CHUNK, S)
    cp_x0, cp_x1, cp_x2 = (
        pltpu.make_async_copy(x_hbm.at[lo:hi], x_v.at[lo:hi], sem_in.at[i])
        for i, (lo, hi) in enumerate(zip(x_cuts, x_cuts[1:])))
    cp_bwo = pltpu.make_async_copy(bwo_hbm, bwo_v, sem_in.at[3])
    cp_wo = pltpu.make_async_copy(wo_hbm, wo_v, sem_in.at[4])

    def cp_bqkv(s):
        rows = pl.ds(pl.multiple_of(s * LANES, LANES), LANES)
        return pltpu.make_async_copy(bqkv_hbm.at[rows], bqkv_v.at[rows],
                                     sem_b.at[s])

    def cp_w(i):
        last = isinstance(i, int) and i == n_late
        n = (n_pair - n_late * ppc if last else ppc) * PW
        rows = pl.ds(pl.multiple_of(i * ppc * PW, PW), n)
        return [pltpu.make_async_copy(src.at[rows], wraw.at[j, rows],
                                      sem_w.at[i, j])
                for j, src in enumerate((wq_hbm, wk_hbm, wv_hbm))]

    for s in range(n_slab):
        cp_bqkv(s).start()
    cp_x0.start()
    for ref in buf_b:
        ref[...] = jnp.zeros(ref.shape, ref.dtype)

    def permute_bqkv(s, carry):
        cp_bqkv(s).wait()

        @pl.when(s == n_slab - 1)
        def _():
            cp_x1.start()
            cp_x2.start()
            cp_bwo.start()
            for cp in cp_w(0):
                cp.start()

        rows = pl.ds(pl.multiple_of(s * LANES, LANES), LANES)
        slab[0:3 * D, :] = bqkv_v[rows, :].astype(F32).T
        for part in range(3):
            for d in range(bdh):
                r0 = part * D + d * B_HEADS
                bqkv_p[s, r0:r0 + B_HEADS, :] = slab[
                    pl.ds(part * D + d, B_HEADS, stride=bdh), :].astype(BF16)
        return carry

    lax.fori_loop(0, n_slab, permute_bqkv, 0)
    cp_x0.wait()

    bscale = bdh ** -0.5
    gate = gate_ref[...].astype(F32).reshape(1, D)

    def b_project(t0, dst, prev, is_first):
        for j in range(3):
            w = jnp.concatenate(
                [bqkv_p[s, j * D:(j + 1) * D, :] for s in range(n_slab)], axis=1)
            y = _dot_nt(x_v[pl.ds(t0, B_CHUNK), :], w)
            for s in range(n_slab):
                t = y[:, s * LANES:(s + 1) * LANES]
                if j == 0:
                    dst[j][s] = t
                    continue
                halo = prev[j][s, B_CHUNK:, :]
                if is_first is not None:
                    halo = jnp.where(
                        is_first, jnp.broadcast_to(t[0:1], halo.shape), halo)
                dst[j][s, 0:B_PAD, :] = halo
                dst[j][s, B_PAD:, :] = t
            yield

    def b_attend(t0, src):
        q_s, k_s, v_s = src
        for r in range(0, B_CHUNK, B_SUB):
            qs = [q_s[s, r:r + B_SUB, :] for s in range(n_slab)]
            logits = []
            for w in range(B_WIN):
                o = B_PAD + r - w * B_DIL
                acc = qs[0] * k_s[0, o:o + B_SUB, :]
                for s in range(1, n_slab):
                    acc = acc + qs[s] * k_s[s, o:o + B_SUB, :]
                acc = acc + pltpu.roll(acc, 64, 1)
                acc = acc + pltpu.roll(acc, 32, 1)
                if r < w * B_DIL:
                    pos = t0 + r + lax.broadcasted_iota(
                        jnp.int32, (B_SUB, LANES), 0)
                    acc = jnp.where(pos >= w * B_DIL, acc, NEG / bscale)
                logits.append(acc)
            mx = functools.reduce(jnp.maximum, logits)
            es = [jnp.exp2((l - mx) * (bscale * LOG2E)) for l in logits]
            inv = 1.0 / functools.reduce(jnp.add, es)
            cols = []
            for s in range(n_slab):
                acc = None
                for w in range(B_WIN):
                    o = B_PAD + r - w * B_DIL
                    t = es[w] * v_s[s, o:o + B_SUB, :]
                    acc = t if acc is None else acc + t
                cols.append((acc * inv).astype(BF16))
            ob_v[pl.ds(t0 + r, B_SUB), :] = jnp.concatenate(cols, axis=1)
            if (r // B_SUB) % 2:
                yield

    def prepare(pairs):
        for p in pairs:
            tok = pl.ds(pl.multiple_of(p * (S // n_pair), S // n_pair),
                        S // n_pair)
            g = jax.nn.sigmoid(jnp.sum(x_v[tok, :].astype(F32) * gate,
                                       axis=-1, keepdims=True))
            g_v[tok, :] = jnp.broadcast_to(g, (S // n_pair, LANES))
            rows = pl.ds(pl.multiple_of(p * PW, PW), PW)
            qpre[p] = _dot_nt(xt_v[...], wraw[0, rows, :])
            yield
            for j in range(3):
                w_v[p, :, j * PW:(j + 1) * PW] = wraw[j, rows, :].T
            yield

    def b_chunks(c, is_first):
        t0 = pl.multiple_of(c * 2 * B_CHUNK, B_CHUNK)
        t1 = pl.multiple_of(t0 + B_CHUNK, B_CHUNK)
        tp = pl.multiple_of(jnp.maximum(t0 - B_CHUNK, 0), B_CHUNK)
        _interleave(b_project(t0, buf_a, buf_b, is_first), b_attend(tp, buf_b))
        _interleave(b_project(t1, buf_b, buf_a, None), b_attend(t0, buf_a))

    def early_body(c, carry):
        b_chunks(c, c == 0)

        @pl.when(c == 0)
        def _():
            cp_x1.wait()

        return carry

    lax.fori_loop(0, N_EARLY, early_body, 0)
    cp_x2.wait()
    for cp in cp_w(1):
        cp.start()
    def gather_tail(i, carry):
        parts = []
        for u in range(2):
            r = pl.multiple_of((2 * i + u + 1) * seg - 2 * PRE, 2 * PRE)
            parts.append(x_v[pl.ds(r, 2 * PRE), :].astype(F32)[PRE:])
        xt_v[pl.ds(pl.multiple_of(i * 2 * PRE, 2 * PRE), 2 * PRE), :] = (
            jnp.concatenate(parts, axis=0).astype(BF16))
        return carry

    lax.fori_loop(0, n_seg // 2, gather_tail, 0, unroll=8)

    def permute_bwo(s):
        cols = pl.ds(pl.multiple_of(s * LANES, LANES), LANES)
        slab[0:D, :] = bwo_v[:, cols].astype(F32)
        for d in range(bdh):
            bwo_p[d * B_HEADS:(d + 1) * B_HEADS, cols] = slab[
                pl.ds(d, B_HEADS, stride=bdh), :].astype(BF16)

    cp_bwo.wait()

    def late_body(i, carry):
        for cp in cp_w(i):
            cp.wait()

        @pl.when(i + 2 < n_late)
        def _():
            for cp in cp_w(i + 2):
                cp.start()

        @pl.when(i + 2 == n_late)
        def _():
            for cp in cp_w(n_late):
                cp.start()
            cp_wo.start()

        permute_bwo(jnp.minimum(i, n_slab - 1))
        _interleave(prepare([i * ppc + u for u in range(ppc)]))
        b_chunks(i + N_EARLY, None)
        return carry

    lax.fori_loop(0, n_late, late_body, 0)

    for cp in cp_w(n_late):
        cp.wait()
    _interleave(prepare(range(n_late * ppc, n_pair)),
                b_attend(S - B_CHUNK, buf_b))
    cp_wo.wait()

    scale = dh ** -0.5

    def step(s, mem):
        r0 = pl.multiple_of(s * seg, seg)
        h = jnp.concatenate([mem, x_v[pl.ds(r0, seg), :].astype(F32)], axis=0)

        row = lax.broadcasted_iota(jnp.int32, (L, 2 * L), 0)
        col = lax.broadcasted_iota(jnp.int32, (L, 2 * L), 1)
        first = col < L
        visible = (row < M) | (row >= jnp.where(first, col, col - L))
        lo = lax.broadcasted_iota(jnp.int32, (L, PW), 1) < dh

        def block_diag(t):
            return jnp.concatenate(
                [jnp.where(lo, t, 0.0), jnp.where(lo, 0.0, t)],
                axis=0).astype(BF16)

        def project(p):
            q = jnp.concatenate(
                [_dot(h[:L - PRE], w_v[p, :, :PW]),
                 qpre[p, pl.ds(pl.multiple_of(s * PRE, PRE), PRE), :]], axis=0)
            kv = _dot(h, w_v[p, :, PW:])
            return q, block_diag(kv[:, :PW]), block_diag(kv[:, PW:])

        def scores(q, kb):
            sc = jnp.where(visible, _dot_nt(q, kb) * scale, NEG)
            ma = jnp.max(jnp.where(first, sc, -jnp.inf), axis=-1, keepdims=True)
            mb = jnp.max(jnp.where(first, -jnp.inf, sc), axis=-1, keepdims=True)
            e = jnp.exp(sc - jnp.where(first, ma, mb))
            sa = jnp.sum(jnp.where(first, e, 0.0), axis=-1, keepdims=True)
            sb = jnp.sum(jnp.where(first, 0.0, e), axis=-1, keepdims=True)
            return e * jnp.where(first, 1.0 / sa, 1.0 / sb)

        proj, prob, outs = {}, {}, {}
        acc = None

        def out_proj(acc, pairs):
            for p in pairs:
                y = _dot(outs[p], wo_v[p * PW:(p + 1) * PW, :])
                acc = y if acc is None else acc + y
            return acc

        for t in range(n_pair + 2):
            if t < n_pair:
                proj[t] = project(t)
            if t == n_pair:
                acc = out_proj(acc, range(0, n_pair // 4))
            if 0 <= t - 1 < n_pair:
                prob[t - 1] = scores(proj[t - 1][0], proj[t - 1][1])
            if t == n_pair + 1:
                acc = out_proj(acc, range(n_pair // 4, n_pair - 4))
            if 0 <= t - 2 < n_pair:
                outs[t - 2] = _dot(prob[t - 2], proj[t - 2][2])
        acc = out_proj(acc, range(n_pair - 4, n_pair))

        b = _dot(ob_v[pl.ds(r0, seg), :], bwo_p[...])
        g = jnp.concatenate([g_v[pl.ds(r0, seg), :]] * n_slab, axis=1)
        out_v[pl.ds(r0, seg), :] = (
            g * acc[M:] + (1.0 - g) * b).astype(out_v.dtype)
        pltpu.make_async_copy(out_v.at[pl.ds(r0, seg)],
                              out_hbm.at[pl.ds(r0, seg)], sem_out.at[0]).start()
        return acc[:M]

    lax.fori_loop(0, n_seg, step, mem0_ref[...].astype(F32), unroll=UNROLL)
    pltpu.make_async_copy(out_v, out_v, sem_out.at[0]).wait()


@functools.partial(jax.jit, static_argnames=("A_seg_len",))
def pallas_gated_mix__memory_aug_recurrent_mem_tr__sliding_local_dilated__prompt_kernel(
    A_x: jax.Array,
    A_mem0: jax.Array,
    A_Wq: jax.Array,
    A_Wk: jax.Array,
    A_Wv: jax.Array,
    A_Wo: jax.Array,
    A_seg_len: int,
    B_x: jax.Array,
    B_wqkv: jax.Array,
    B_wo: jax.Array,
    gate_w: jax.Array,
):
    del B_x
    _, S, D = A_x.shape
    _, H, Dh = A_Wq.shape
    M = A_mem0.shape[1]
    seg = int(A_seg_len)
    n_pair = H // 2
    n_slab = D // LANES
    n_chunk = S // (2 * B_CHUNK)

    def by_head(w):
        return jnp.transpose(w, (1, 2, 0)).reshape(H * Dh, D)

    qkv_buf = [pltpu.VMEM((n_slab, B_CHUNK, LANES), F32),
               pltpu.VMEM((n_slab, B_CHUNK + B_PAD, LANES), F32),
               pltpu.VMEM((n_slab, B_CHUNK + B_PAD, LANES), F32)]
    hbm = pl.BlockSpec(memory_space=pl.ANY)
    vmem = pl.BlockSpec(memory_space=pltpu.VMEM)
    out = pl.pallas_call(
        functools.partial(_kernel, seg=seg, n_heads=H, dh=Dh),
        out_shape=jax.ShapeDtypeStruct((S, D), A_x.dtype),
        in_specs=[hbm, vmem, hbm, hbm, hbm, hbm, hbm, hbm, vmem],
        out_specs=hbm,
        scratch_shapes=[
            pltpu.VMEM((S, D), BF16),
            pltpu.VMEM((S // seg * PRE, D), BF16),
            pltpu.VMEM((3, H * Dh, D), BF16),
            pltpu.VMEM((n_pair, D, 6 * Dh), BF16),
            pltpu.VMEM((H * Dh, D), BF16),
            pltpu.VMEM((D, 3 * D), BF16),
            pltpu.VMEM((D, D), BF16),
            pltpu.VMEM((3 * D + B_HEADS, LANES), F32),
            pltpu.VMEM((n_slab, 3 * D, LANES), BF16),
            pltpu.VMEM((D, D), BF16),
            *qkv_buf, *qkv_buf,
            pltpu.VMEM((S, LANES), F32),
            pltpu.VMEM((S, D), BF16),
            pltpu.VMEM((n_pair, S // seg * PRE, 2 * Dh), F32),
            pltpu.VMEM((S, D), A_x.dtype),
            pltpu.SemaphoreType.DMA((5,)),
            pltpu.SemaphoreType.DMA((n_slab,)),
            pltpu.SemaphoreType.DMA((n_chunk - N_EARLY + 1, 3)),
            pltpu.SemaphoreType.DMA((1,)),
        ],
        compiler_params=pltpu.CompilerParams(
            vmem_limit_bytes=110 * 1024 * 1024),
    )(A_x.reshape(S, D), A_mem0.reshape(M, D), by_head(A_Wq), by_head(A_Wk),
      by_head(A_Wv), A_Wo.reshape(H * Dh, D), B_wqkv, B_wo,
      gate_w)
    return out.reshape(1, S, D)
```

```python
import functools

import jax
import jax.numpy as jnp
from jax import lax
import jax.experimental.pallas as pl
import jax.experimental.pallas.tpu as pltpu

F32 = jnp.float32
BF16 = jnp.bfloat16
LANES = 128
NEG = -1000000000.0
LOG2E = 1.4426950408889634

B_HEADS = 32
B_WIN = 8
B_DIL = 2
B_PAD = 16
B_CHUNK = 128
B_SUB = 32
N_EARLY = 2
PRE = 8
UNROLL = 4


def _dot(a, b):
    return lax.dot_general(a, b, (((1,), (0,)), ((), ())),
                           preferred_element_type=F32)


def _dot_nt(a, b):
    return lax.dot_general(a, b, (((1,), (1,)), ((), ())),
                           preferred_element_type=F32)


def _interleave(*stages):
    stages = list(stages)
    while stages:
        for g in list(stages):
            if next(g, _DONE) is _DONE:
                stages.remove(g)


_DONE = object()


def _kernel(x_hbm, mem0_ref, wq_hbm, wk_hbm, wv_hbm, wo_hbm, bqkv_hbm, bwo_hbm,
            gate_ref, out_hbm,
            x_v, xt_v, wraw, w_v, wo_v, bqkv_v, bwo_v, slab, bqkv_p, bwo_p,
            q_a, k_a, v_a, q_b, k_b, v_b, g_v, ob_v, qpre, out_v,
            sem_in, sem_b, sem_w, sem_out,
            *, seg, n_heads, dh):
    S, D = x_v.shape
    M = mem0_ref.shape[0]
    L = M + seg
    n_seg = S // seg
    n_pair = n_heads // 2
    PW = 2 * dh
    n_slab = D // LANES
    bdh = D // B_HEADS
    n_chunk = S // (2 * B_CHUNK)
    n_late = n_chunk - N_EARLY
    assert n_late >= n_slab
    ppc = n_pair // n_late
    buf_a, buf_b = (q_a, k_a, v_a), (q_b, k_b, v_b)

    x_cuts = (0, 2 * B_CHUNK, 2 * N_EARLY * B_CHUNK, S)
    cp_x0, cp_x1, cp_x2 = (
        pltpu.make_async_copy(x_hbm.at[lo:hi], x_v.at[lo:hi], sem_in.at[i])
        for i, (lo, hi) in enumerate(zip(x_cuts, x_cuts[1:])))
    cp_bwo = pltpu.make_async_copy(bwo_hbm, bwo_v, sem_in.at[3])

    def cp_bqkv(s):
        rows = pl.ds(pl.multiple_of(s * LANES, LANES), LANES)
        return pltpu.make_async_copy(bqkv_hbm.at[rows], bqkv_v.at[rows],
                                     sem_b.at[s])

    def cp_wo(i):
        n = n_pair * PW // n_late
        assert n * n_late == n_pair * PW
        rows = pl.ds(pl.multiple_of(i * n, n), n)
        return pltpu.make_async_copy(wo_hbm.at[rows], wo_v.at[rows],
                                     sem_in.at[4])

    def cp_w(i):
        last = isinstance(i, int) and i == n_late
        n = (n_pair - n_late * ppc if last else ppc) * PW
        rows = pl.ds(pl.multiple_of(i * ppc * PW, PW), n)
        return [pltpu.make_async_copy(src.at[rows], wraw.at[j, rows],
                                      sem_w.at[i, j])
                for j, src in enumerate((wq_hbm, wk_hbm, wv_hbm))]

    for s in range(n_slab):
        cp_bqkv(s).start()
    cp_x0.start()
    for ref in buf_b:
        ref[...] = jnp.zeros(ref.shape, ref.dtype)

    def permute_bqkv(s, carry):
        cp_bqkv(s).wait()

        @pl.when(s == n_slab - 1)
        def _():
            cp_x1.start()
            cp_x2.start()
            cp_bwo.start()
            for cp in cp_w(0):
                cp.start()

        rows = pl.ds(pl.multiple_of(s * LANES, LANES), LANES)
        slab[0:3 * D, :] = bqkv_v[rows, :].astype(F32).T
        for part in range(3):
            for d in range(bdh):
                r0 = part * D + d * B_HEADS
                bqkv_p[s, r0:r0 + B_HEADS, :] = slab[
                    pl.ds(part * D + d, B_HEADS, stride=bdh), :].astype(BF16)
        return carry

    lax.fori_loop(0, n_slab, permute_bqkv, 0)
    cp_x0.wait()

    bscale = bdh ** -0.5
    gate = gate_ref[...].astype(F32).reshape(1, D)

    def b_project(t0, dst, prev, is_first):
        for j in range(3):
            w = jnp.concatenate(
                [bqkv_p[s, j * D:(j + 1) * D, :] for s in range(n_slab)], axis=1)
            y = _dot_nt(x_v[pl.ds(t0, B_CHUNK), :], w)
            for s in range(n_slab):
                t = y[:, s * LANES:(s + 1) * LANES]
                if j == 0:
                    dst[j][s] = t
                    continue
                halo = prev[j][s, B_CHUNK:, :]
                if is_first is not None:
                    halo = jnp.where(
                        is_first, jnp.broadcast_to(t[0:1], halo.shape), halo)
                dst[j][s, 0:B_PAD, :] = halo
                dst[j][s, B_PAD:, :] = t
            yield

    def b_attend(t0, src):
        q_s, k_s, v_s = src
        for r in range(0, B_CHUNK, B_SUB):
            qs = [q_s[s, r:r + B_SUB, :] for s in range(n_slab)]
            logits = []
            for w in range(B_WIN):
                o = B_PAD + r - w * B_DIL
                acc = qs[0] * k_s[0, o:o + B_SUB, :]
                for s in range(1, n_slab):
                    acc = acc + qs[s] * k_s[s, o:o + B_SUB, :]
                acc = acc + pltpu.roll(acc, 64, 1)
                acc = acc + pltpu.roll(acc, 32, 1)
                if r < w * B_DIL:
                    pos = t0 + r + lax.broadcasted_iota(
                        jnp.int32, (B_SUB, LANES), 0)
                    acc = jnp.where(pos >= w * B_DIL, acc, NEG / bscale)
                logits.append(acc)
            mx = functools.reduce(jnp.maximum, logits)
            es = [jnp.exp2((l - mx) * (bscale * LOG2E)) for l in logits]
            inv = 1.0 / functools.reduce(jnp.add, es)
            cols = []
            for s in range(n_slab):
                acc = None
                for w in range(B_WIN):
                    o = B_PAD + r - w * B_DIL
                    t = es[w] * v_s[s, o:o + B_SUB, :]
                    acc = t if acc is None else acc + t
                cols.append((acc * inv).astype(BF16))
            ob_v[pl.ds(t0 + r, B_SUB), :] = jnp.concatenate(cols, axis=1)
            if (r // B_SUB) % 2:
                yield

    def prepare(pairs):
        for p in pairs:
            tok = pl.ds(pl.multiple_of(p * (S // n_pair), S // n_pair),
                        S // n_pair)
            g = jax.nn.sigmoid(jnp.sum(x_v[tok, :].astype(F32) * gate,
                                       axis=-1, keepdims=True))
            g_v[tok, :] = jnp.broadcast_to(g, (S // n_pair, LANES))
            rows = pl.ds(pl.multiple_of(p * PW, PW), PW)
            qpre[p] = _dot_nt(xt_v[...], wraw[0, rows, :])
            yield
            for j in range(3):
                w_v[p, :, j * PW:(j + 1) * PW] = wraw[j, rows, :].T
            yield

    def b_chunks(c, is_first):
        t0 = pl.multiple_of(c * 2 * B_CHUNK, B_CHUNK)
        t1 = pl.multiple_of(t0 + B_CHUNK, B_CHUNK)
        tp = pl.multiple_of(jnp.maximum(t0 - B_CHUNK, 0), B_CHUNK)
        _interleave(b_project(t0, buf_a, buf_b, is_first), b_attend(tp, buf_b))
        _interleave(b_project(t1, buf_b, buf_a, None), b_attend(t0, buf_a))

    def early_body(c, carry):
        b_chunks(c, c == 0)

        @pl.when(c == 0)
        def _():
            cp_x1.wait()

        return carry

    lax.fori_loop(0, N_EARLY, early_body, 0)
    cp_x2.wait()
    for cp in cp_w(1):
        cp.start()
    def gather_tail(i, carry):
        parts = []
        for u in range(2):
            r = pl.multiple_of((2 * i + u + 1) * seg - 2 * PRE, 2 * PRE)
            parts.append(x_v[pl.ds(r, 2 * PRE), :].astype(F32)[PRE:])
        xt_v[pl.ds(pl.multiple_of(i * 2 * PRE, 2 * PRE), 2 * PRE), :] = (
            jnp.concatenate(parts, axis=0).astype(BF16))
        return carry

    lax.fori_loop(0, n_seg // 2, gather_tail, 0, unroll=8)

    def permute_bwo(s):
        cols = pl.ds(pl.multiple_of(s * LANES, LANES), LANES)
        slab[0:D, :] = bwo_v[:, cols].astype(F32)
        for d in range(bdh):
            bwo_p[d * B_HEADS:(d + 1) * B_HEADS, cols] = slab[
                pl.ds(d, B_HEADS, stride=bdh), :].astype(BF16)

    cp_bwo.wait()

    def late_body(i, carry):
        for cp in cp_w(i):
            cp.wait()

        @pl.when(i + 2 < n_late)
        def _():
            for cp in cp_w(i + 2):
                cp.start()

        @pl.when(i + 2 == n_late)
        def _():
            for cp in cp_w(n_late):
                cp.start()

        cp_wo(i).start()
        permute_bwo(jnp.minimum(i, n_slab - 1))
        _interleave(prepare([i * ppc + u for u in range(ppc)]))
        b_chunks(i + N_EARLY, None)
        return carry

    lax.fori_loop(0, n_late, late_body, 0)

    for cp in cp_w(n_late):
        cp.wait()
    _interleave(prepare(range(n_late * ppc, n_pair)),
                b_attend(S - B_CHUNK, buf_b))
    pltpu.make_async_copy(wo_v, wo_v, sem_in.at[4]).wait()

    scale = dh ** -0.5

    def step(s, mem):
        r0 = pl.multiple_of(s * seg, seg)
        h = jnp.concatenate([mem, x_v[pl.ds(r0, seg), :].astype(F32)], axis=0)

        row = lax.broadcasted_iota(jnp.int32, (L, 2 * L), 0)
        col = lax.broadcasted_iota(jnp.int32, (L, 2 * L), 1)
        first = col < L
        visible = (row < M) | (row >= jnp.where(first, col, col - L))
        lo = lax.broadcasted_iota(jnp.int32, (L, PW), 1) < dh

        def block_diag(t):
            return jnp.concatenate(
                [jnp.where(lo, t, 0.0), jnp.where(lo, 0.0, t)],
                axis=0).astype(BF16)

        def project(p):
            q = jnp.concatenate(
                [_dot(h[:L - PRE], w_v[p, :, :PW]),
                 qpre[p, pl.ds(pl.multiple_of(s * PRE, PRE), PRE), :]], axis=0)
            kv = _dot(h, w_v[p, :, PW:])
            return q, block_diag(kv[:, :PW]), block_diag(kv[:, PW:])

        def scores(q, kb):
            sc = jnp.where(visible, _dot_nt(q, kb) * scale, NEG)
            ma = jnp.max(jnp.where(first, sc, -jnp.inf), axis=-1, keepdims=True)
            mb = jnp.max(jnp.where(first, -jnp.inf, sc), axis=-1, keepdims=True)
            e = jnp.exp(sc - jnp.where(first, ma, mb))
            sa = jnp.sum(jnp.where(first, e, 0.0), axis=-1, keepdims=True)
            sb = jnp.sum(jnp.where(first, 0.0, e), axis=-1, keepdims=True)
            return e * jnp.where(first, 1.0 / sa, 1.0 / sb)

        proj, prob, outs = {}, {}, {}
        acc = None

        def out_proj(acc, pairs):
            for p in pairs:
                y = _dot(outs[p], wo_v[p * PW:(p + 1) * PW, :])
                acc = y if acc is None else acc + y
            return acc

        for t in range(n_pair + 2):
            if t < n_pair:
                proj[t] = project(t)
            if t == n_pair:
                acc = out_proj(acc, range(0, n_pair // 4))
            if 0 <= t - 1 < n_pair:
                prob[t - 1] = scores(proj[t - 1][0], proj[t - 1][1])
            if t == n_pair + 1:
                acc = out_proj(acc, range(n_pair // 4, n_pair - 4))
            if 0 <= t - 2 < n_pair:
                outs[t - 2] = _dot(prob[t - 2], proj[t - 2][2])
        acc = out_proj(acc, range(n_pair - 4, n_pair))

        b = _dot(ob_v[pl.ds(r0, seg), :], bwo_p[...])
        g = jnp.concatenate([g_v[pl.ds(r0, seg), :]] * n_slab, axis=1)
        out_v[pl.ds(r0, seg), :] = (
            g * acc[M:] + (1.0 - g) * b).astype(out_v.dtype)
        pltpu.make_async_copy(out_v.at[pl.ds(r0, seg)],
                              out_hbm.at[pl.ds(r0, seg)], sem_out.at[0]).start()
        return acc[:M]

    lax.fori_loop(0, n_seg, step, mem0_ref[...].astype(F32), unroll=UNROLL)
    pltpu.make_async_copy(out_v, out_v, sem_out.at[0]).wait()


@functools.partial(jax.jit, static_argnames=("A_seg_len",))
def pallas_gated_mix__memory_aug_recurrent_mem_tr__sliding_local_dilated__prompt_kernel(
    A_x: jax.Array,
    A_mem0: jax.Array,
    A_Wq: jax.Array,
    A_Wk: jax.Array,
    A_Wv: jax.Array,
    A_Wo: jax.Array,
    A_seg_len: int,
    B_x: jax.Array,
    B_wqkv: jax.Array,
    B_wo: jax.Array,
    gate_w: jax.Array,
):
    del B_x
    _, S, D = A_x.shape
    _, H, Dh = A_Wq.shape
    M = A_mem0.shape[1]
    seg = int(A_seg_len)
    n_pair = H // 2
    n_slab = D // LANES
    n_chunk = S // (2 * B_CHUNK)

    def by_head(w):
        return jnp.transpose(w, (1, 2, 0)).reshape(H * Dh, D)

    qkv_buf = [pltpu.VMEM((n_slab, B_CHUNK, LANES), F32),
               pltpu.VMEM((n_slab, B_CHUNK + B_PAD, LANES), F32),
               pltpu.VMEM((n_slab, B_CHUNK + B_PAD, LANES), F32)]
    hbm = pl.BlockSpec(memory_space=pl.ANY)
    vmem = pl.BlockSpec(memory_space=pltpu.VMEM)
    out = pl.pallas_call(
        functools.partial(_kernel, seg=seg, n_heads=H, dh=Dh),
        out_shape=jax.ShapeDtypeStruct((S, D), A_x.dtype),
        in_specs=[hbm, vmem, hbm, hbm, hbm, hbm, hbm, hbm, vmem],
        out_specs=hbm,
        scratch_shapes=[
            pltpu.VMEM((S, D), BF16),
            pltpu.VMEM((S // seg * PRE, D), BF16),
            pltpu.VMEM((3, H * Dh, D), BF16),
            pltpu.VMEM((n_pair, D, 6 * Dh), BF16),
            pltpu.VMEM((H * Dh, D), BF16),
            pltpu.VMEM((D, 3 * D), BF16),
            pltpu.VMEM((D, D), BF16),
            pltpu.VMEM((3 * D + B_HEADS, LANES), F32),
            pltpu.VMEM((n_slab, 3 * D, LANES), BF16),
            pltpu.VMEM((D, D), BF16),
            *qkv_buf, *qkv_buf,
            pltpu.VMEM((S, LANES), F32),
            pltpu.VMEM((S, D), BF16),
            pltpu.VMEM((n_pair, S // seg * PRE, 2 * Dh), F32),
            pltpu.VMEM((S, D), A_x.dtype),
            pltpu.SemaphoreType.DMA((5,)),
            pltpu.SemaphoreType.DMA((n_slab,)),
            pltpu.SemaphoreType.DMA((n_chunk - N_EARLY + 1, 3)),
            pltpu.SemaphoreType.DMA((1,)),
        ],
        compiler_params=pltpu.CompilerParams(
            vmem_limit_bytes=110 * 1024 * 1024),
    )(A_x.reshape(S, D), A_mem0.reshape(M, D), by_head(A_Wq), by_head(A_Wk),
      by_head(A_Wv), A_Wo.reshape(H * Dh, D), B_wqkv, B_wo,
      gate_w)
    return out.reshape(1, S, D)
```
